```python
import os as _os
_os.environ.setdefault("JAX_PLATFORMS", "cpu")
import jax
import jax.numpy as jnp

def _softmax(x, axis=-1):
    return jax.nn.softmax(x, axis=axis)
def _gelu(x):
    return jax.nn.gelu(x, approximate=True)
def _silu(x):
    return jax.nn.silu(x)
def _sigmoid(x):
    return jax.nn.sigmoid(x)
def _layernorm(x, axis=-1, eps=1e-5):
    m = jnp.mean(x, axis=axis, keepdims=True)
    v = jnp.var(x, axis=axis, keepdims=True)
    return (x - m) / jnp.sqrt(v + eps)
def _scatter_add(tgt, idx, src, axis=0):
    return tgt.at[idx].add(src)
def _segment_sum(src, seg, n):
    return jax.ops.segment_sum(src, seg, n)
class _Rng:
    def __init__(self, key):
        self._k = key
    def _next(self):
        self._k, sub = jax.random.split(self._k)
        return sub
    def normal(self, shape):
        return jax.random.normal(self._next(), shape, dtype=jnp.bfloat16)
    def randint(self, lo, hi, shape):
        return jax.random.randint(self._next(), shape, lo, hi, dtype=jnp.int32)
    def uniform(self, shape, lo=0.0, hi=1.0):
        return jax.random.uniform(self._next(), shape, jnp.bfloat16, lo, hi)
    def permutation(self, n):
        return jax.random.permutation(self._next(), n)


kernel_name = 'recurrent_scan__linear_attn_block__geglu_ffn__prompt'

def setup_inputs():
    _rng = _Rng(jax.random.key(int.from_bytes(__import__("os").urandom(4), "little")))
    _w = (lambda a: (lambda t: t.astype(jnp.bfloat16) if jnp.issubdtype(t.dtype, jnp.floating) else t)(jnp.asarray(a)))
    def _A_setup():
        B, S, D = 1, 2048, 512
        return {
            "x": _w((lambda *s: _rng.normal(s) * 0.05)(B, S, D)),
            "wqkv": _w((lambda *s: _rng.normal(s) * 0.05)(D, 3 * D)),
            "wo": _w((lambda *s: _rng.normal(s) * 0.05)(D, D)),
        }
    _A_in = _A_setup()

    def _B_setup():
        B, S, D, F = 1, 2048, 512, 1792
        return {
            "x": _w((lambda *s: _rng.normal(s) * 0.05)(B, S, D)),
            "w_gate": _w((lambda *s: _rng.normal(s) * 0.05)(D, F)),
            "w_up": _w((lambda *s: _rng.normal(s) * 0.05)(D, F)),
            "w_down": _w((lambda *s: _rng.normal(s) * 0.05)(F, D)),
        }
    _B_in = _B_setup()

    return {
        "A_x": _A_in["x"],
        "A_wqkv": _A_in["wqkv"],
        "A_wo": _A_in["wo"],
        "B_x": _B_in["x"],
        "B_w_gate": _B_in["w_gate"],
        "B_w_up": _B_in["w_up"],
        "B_w_down": _B_in["w_down"],
    }

def reference(A_x, A_wqkv, A_wo, B_x, B_w_gate, B_w_up, B_w_down):
    def _A_ref(x, wqkv, wo):
        B, S, D = x.shape
        H = 32; Dh = D // H
        qkv = (lambda x, *d: x.transpose(*d))((x @ wqkv).reshape(B, S, 3, H, Dh), 2, 0, 3, 1, 4)
        q, k, v = qkv[0], qkv[1], qkv[2]
        phi = lambda t: jnp.where(t > 0, t + 1, jnp.exp(t)) + 1e-6
        pq, pk = phi(q), phi(k)
        kv = jnp.einsum("bhsd,bhse->bhde", pk, v)
        z = jnp.einsum("bhsd->bhd", pk)
        num = jnp.einsum("bhqd,bhde->bhqe", pq, kv)
        den = jnp.einsum("bhqd,bhd->bhq", pq, z)[..., None] + 1e-6
        o = num / den
        return (lambda x, *d: x.transpose(*d))(o, 0, 2, 1, 3).reshape(B, S, D) @ wo

    def _B_ref(x, w_gate, w_up, w_down):
        return (_gelu(x @ w_gate) * (x @ w_up)) @ w_down

    x = A_x
    xn = _layernorm(x, axis=-1)
    s = _A_ref(xn, A_wqkv, A_wo)
    g = _silu(_B_ref(xn, B_w_gate, B_w_up, B_w_down))
    return x + s * g
```

```python
import functools
import jax
import jax.numpy as jnp
from jax import lax
import jax.experimental.pallas as pl
import jax.experimental.pallas.tpu as pltpu

S, D, F, H = 2048, 512, 1792, 32
DH = D // H
BF = jnp.bfloat16
F32 = jnp.float32
NT = (((1,), (1,)), ((), ()))


def _phi(t):
    return jnp.where(t > 0, t + 1.0, jnp.exp(t)) + 1e-6


def _gelu_mul(x, up):
    c0 = 0.7978845608028654
    c1 = 0.7978845608028654 * 0.044715
    t = jnp.tanh(x * (c0 + c1 * (x * x)))
    return (0.5 * x * up) * (1.0 + t)


def make(XC=(256, 512, 1280), KSUB=512, QT=512, TM=512, SUBS=(512,), NLX=None, stop=None, waitall=False, noffn=False, delay=0):
    assert sum(XC) == S
    xoff = [sum(XC[:i]) for i in range(len(XC))]
    NX = len(XC)
    NL = S // TM
    assert sum(SUBS) == TM
    NS = len(SUBS)
    soff = [sum(SUBS[:i]) for i in range(NS)]

    def kernel(x_hbm, wqkv_hbm, wo_hbm, wg_hbm, wu_hbm, wd_hbm, o_hbm,
               x_v, wqkv_v, wo_v, wg_v, wu_v, wd_v, wkt_v, tmp_v, wqp_v, xn_v, pkt_v, g_acc, z_acc, m_v,
               a_v, obuf, wsem, osem):
        def xcopy(i):
            return pltpu.make_async_copy(x_hbm.at[pl.ds(xoff[i], XC[i])], x_v.at[pl.ds(xoff[i], XC[i])], wsem.at[7 + i])
        wk_c = pltpu.make_async_copy(wqkv_hbm.at[:, pl.ds(D, D)], wqkv_v.at[:, pl.ds(D, D)], wsem.at[0])
        wq_c = pltpu.make_async_copy(wqkv_hbm.at[:, pl.ds(0, D)], wqkv_v.at[:, pl.ds(0, D)], wsem.at[1])
        wv_c = pltpu.make_async_copy(wqkv_hbm.at[:, pl.ds(2 * D, D)], wqkv_v.at[:, pl.ds(2 * D, D)], wsem.at[2])
        wo_c = pltpu.make_async_copy(wo_hbm, wo_v, wsem.at[3])
        wg_c = pltpu.make_async_copy(wg_hbm, wg_v, wsem.at[4])
        wu_c = pltpu.make_async_copy(wu_hbm, wu_v, wsem.at[5])
        wd_c = pltpu.make_async_copy(wd_hbm, wd_v, wsem.at[6])
        xcopy(0).start()
        wk_c.start()
        for i in range(1, NX):
            xcopy(i).start()
        for c in ((wq_c, wv_c, wo_c) if noffn else (wq_c, wv_c, wo_c, wg_c, wu_c, wd_c)):
            c.start()

        def subtiles(i):
            out = []
            o = xoff[i]
            while o < xoff[i] + XC[i]:
                n = min(KSUB, xoff[i] + XC[i] - o)
                out.append((o, n))
                o += n
            return out

        def ln(o, n):
            x = x_v[o:o + n, :].astype(F32)
            mu = jnp.mean(x, axis=-1, keepdims=True)
            xc = x - mu
            var = jnp.mean(xc * xc, axis=-1, keepdims=True)
            xn_v[o:o + n, :] = (xc * lax.rsqrt(var + 1e-5)).astype(BF)

        def kpart(o, n):
            kt = lax.dot_general(wkt_v[...], xn_v[o:o + n, :], NT, preferred_element_type=F32)
            pkt = _phi(kt)
            zp = pkt[:, 0:128]
            for c in range(1, n // 128):
                zp = zp + pkt[:, c * 128:(c + 1) * 128]
            if o == 0:
                z_acc[...] = zp
            else:
                z_acc[...] += zp
            pkt_v[:, o:o + n] = pkt.astype(BF)

        def gpart(o, n):
            gp = jnp.dot(pkt_v[:, o:o + n], xn_v[o:o + n, :], preferred_element_type=F32)
            for cb in range(4):
                if o == 0:
                    g_acc[cb] = gp[:, cb * 128:(cb + 1) * 128]
                else:
                    g_acc[cb] += gp[:, cb * 128:(cb + 1) * 128]

        if waitall:
            wd_c.wait()
        xcopy(0).wait()
        wk_c.wait()
        for (o, n) in subtiles(0):
            ln(o, n)
        wkt_v[...] = wqkv_v[:, D:2 * D].astype(F32).T.astype(BF)
        pend = None
        for i in range(NX):
            if i > 0:
                xcopy(i).wait()
                for (o, n) in subtiles(i):
                    ln(o, n)
            for (o, n) in subtiles(i):
                if pend is not None:
                    gpart(*pend)
                kpart(o, n)
                pend = (o, n)

        if delay:
            def dbody(i, carry):
                tmp_v[0] = jnp.dot(xn_v[0:512, :], wkt_v[:, 0:128], preferred_element_type=F32) + i.astype(F32)
                return carry
            lax.fori_loop(0, delay, dbody, 0)
        wq_c.wait()
        wv_c.wait()
        wo_c.wait()
        if stop == 'C':
            (None if noffn else (wg_c.wait(), wu_c.wait(), (None if waitall else wd_c.wait())))
            return
        for cb in range(4):
            tmp_v[cb] = wqkv_v[cb * 128:(cb + 1) * 128, 0:D].astype(F32).T
        for j in range(DH):
            for cb in range(4):
                wqp_v[j * H:(j + 1) * H, cb * 128:(cb + 1) * 128] = tmp_v[cb, pl.ds(j, H, stride=DH), :].astype(BF)
        gpart(*pend)
        zperm = jnp.concatenate([z_acc[pl.ds(j, H, stride=DH), :] for j in range(DH)], axis=0)
        zrow = jnp.sum(zperm.T, axis=0, keepdims=True)

        def qpart(o, n):
            q = lax.dot_general(xn_v[o:o + n, :], wqp_v[...], NT, preferred_element_type=F32)
            pq = _phi(q)
            t = pq * zrow
            u = (t[:, 0:128] + t[:, 128:256]) + (t[:, 256:384] + t[:, 384:512])
            u = u + pltpu.roll(u, 64, 1)
            u = u + pltpu.roll(u, 32, 1)
            r = 1.0 / (u + 1e-6)
            for b in range(4):
                a_v[o:o + n, b * 128:(b + 1) * 128] = (pq[:, b * 128:(b + 1) * 128] * r).astype(BF)

        rr = lax.broadcasted_iota(jnp.int32, (128, 128), 0) % 8
        cc = lax.broadcasted_iota(jnp.int32, (128, 128), 1) // DH
        mask = rr == cc

        qts = [(o, QT) for o in range(0, S, QT)]
        qpart(*qts[0])
        kvs = []
        for b in range(4):
            gb = jnp.concatenate([
                jnp.concatenate([g_acc[cb, pl.ds(b * 128 + j, 8, stride=DH), :] for j in range(DH)], axis=0)
                for cb in range(4)], axis=1)
            kvb = jnp.dot(gb.astype(BF), wqkv_v[:, 2 * D + b * 128:2 * D + (b + 1) * 128],
                          preferred_element_type=F32)
            kvs.append(jnp.where(mask, kvb, 0.0).astype(BF))
        qpart(*qts[1])
        ms = [jnp.dot(kvs[b], wo_v[b * 128:(b + 1) * 128, :], preferred_element_type=F32) for b in range(4)]
        mperm = jnp.concatenate([ms[b][j * 8:(j + 1) * 8, :] for j in range(DH) for b in range(4)], axis=0)
        m_v[...] = mperm.astype(BF)
        for qt in qts[2:]:
            qpart(*qt)

        wg_c.wait()
        wu_c.wait()
        wd_c.wait()
        if stop == 'D':
            return

        def ocopy(i, s):
            r0 = pl.multiple_of(i * TM + soff[s], 16)
            return pltpu.make_async_copy(obuf.at[pl.ds(r0, SUBS[s])], o_hbm.at[pl.ds(r0, SUBS[s])], osem.at[0])

        def body(i, carry):
            for s in range(NS):
                row = pl.ds(pl.multiple_of(i * TM + soff[s], 16), SUBS[s])
                xn = xn_v[row, :]
                gt = jnp.dot(xn, wg_v[...], preferred_element_type=F32)
                up = jnp.dot(xn, wu_v[...], preferred_element_type=F32)
                h = _gelu_mul(gt, up).astype(BF)
                y = jnp.dot(h, wd_v[...], preferred_element_type=F32)
                hy = 0.5 * y
                g = hy * (1.0 + jnp.tanh(hy))
                sa = jnp.dot(a_v[row, :], m_v[...], preferred_element_type=F32)
                obuf[row, :] = (x_v[row, :].astype(F32) + sa * g).astype(BF)
                ocopy(i, s).start()
            return carry
        nl = NL if NLX is None else NLX
        lax.fori_loop(0, nl, body, 0)
        pltpu.make_async_copy(obuf.at[pl.ds(0, nl * TM)], o_hbm.at[pl.ds(0, nl * TM)], osem.at[0]).wait()

    def fn(A_x, A_wqkv, A_wo, B_x, B_w_gate, B_w_up, B_w_down):
        x2 = A_x.reshape(S, D)
        out = pl.pallas_call(
            kernel,
            out_shape=jax.ShapeDtypeStruct((S, D), BF),
            in_specs=[pl.BlockSpec(memory_space=pl.ANY)] * 6,
            out_specs=pl.BlockSpec(memory_space=pl.ANY),
            scratch_shapes=[
                pltpu.VMEM((S, D), BF),
                pltpu.VMEM((D, 3 * D), BF),
                pltpu.VMEM((D, D), BF),
                pltpu.VMEM((D, F), BF),
                pltpu.VMEM((D, F), BF),
                pltpu.VMEM((F, D), BF),
                pltpu.VMEM((D, D), BF),
                pltpu.VMEM((4, D, 128), F32),
                pltpu.VMEM((D, D), BF),
                pltpu.VMEM((S, D), BF),
                pltpu.VMEM((D, S), BF),
                pltpu.VMEM((4, D, 128), F32),
                pltpu.VMEM((D, 128), F32),
                pltpu.VMEM((D, D), BF),
                pltpu.VMEM((S, D), BF),
                pltpu.VMEM((S, D), BF),
                pltpu.SemaphoreType.DMA((7 + NX,)),
                pltpu.SemaphoreType.DMA((1,)),
            ],
            compiler_params=pltpu.CompilerParams(vmem_limit_bytes=100 * 1024 * 1024),
        )(x2, A_wqkv, A_wo, B_w_gate, B_w_up, B_w_down)
        return out.reshape(1, S, D)
    return fn


_impl = make()


@jax.jit
def pallas_recurrent_scan__linear_attn_block__geglu_ffn__prompt_kernel(
    A_x: jax.Array,
    A_wqkv: jax.Array,
    A_wo: jax.Array,
    B_x: jax.Array,
    B_w_gate: jax.Array,
    B_w_up: jax.Array,
    B_w_down: jax.Array,
):
    return _impl(A_x, A_wqkv, A_wo, B_x, B_w_gate, B_w_up, B_w_down)
```

```python
import jax
import jax.numpy as jnp
from jax import lax
import jax.experimental.pallas as pl
import jax.experimental.pallas.tpu as pltpu

S, D, F, H = 2048, 512, 1792, 32
DH = D // H
BF = jnp.bfloat16
F32 = jnp.float32
U32 = jnp.uint32
NT = (((1,), (1,)), ((), ()))


def _phi(t):
    return jnp.where(t > 0, t + 1.0, jnp.exp(t)) + 1e-6


def _gelu_mul(x, up):
    c0 = 0.7978845608028654
    c1 = 0.7978845608028654 * 0.044715
    t = jnp.tanh(x * (c0 + c1 * (x * x)))
    return (0.5 * x * up) * (1.0 + t)


def _rl(x, k):
    return pltpu.roll(x, k % 128, 1)


def _normalize(pq, zrow):
    n = pq.shape[0]
    lane = lax.broadcasted_iota(jnp.int32, (n, 128), 1)
    b0 = (lane & 1) != 0
    b1 = (lane & 2) != 0
    b2 = (lane & 4) != 0
    b3 = (lane & 8) != 0
    t = pq * zrow
    tb = [t[:, b * 128:(b + 1) * 128] for b in range(4)]
    m01 = jnp.where(b0, tb[0] + _rl(tb[0], 1), tb[1] + _rl(tb[1], -1))
    m23 = jnp.where(b0, tb[2] + _rl(tb[2], 1), tb[3] + _rl(tb[3], -1))
    u = jnp.where(b1, m01 + _rl(m01, 2), m23 + _rl(m23, -2))
    u = u + jnp.where(b2, _rl(u, 4), _rl(u, -4))
    u = u + jnp.where(b3, _rl(u, 8), _rl(u, -8))
    r = 1.0 / (u + 1e-6)
    r01 = jnp.where(b1, r, _rl(r, -2))
    r23 = jnp.where(b1, _rl(r, 2), r)
    rs = [jnp.where(b0, r01, _rl(r01, -1)), jnp.where(b0, _rl(r01, 1), r01),
          jnp.where(b0, r23, _rl(r23, -1)), jnp.where(b0, _rl(r23, 1), r23)]
    return jnp.concatenate([(pq[:, b * 128:(b + 1) * 128] * rs[b]).astype(BF) for b in range(4)], axis=1)


def _dot(a, b):
    return jnp.dot(a, b, preferred_element_type=F32)


def _sum8(x):
    n, c = x.shape
    return jnp.sum(x.reshape(n // 8, 8, c), axis=0)


def make(A=896, E=128, NH=2, LAG=2, KSUB=256, GLN=2, NL=2, P0=512, SA=(256, 128, 128), OSPLIT=4,
         QA=128, Q0=768, WT=(2, 3, 5, 5)):
    TA = sum(SA)
    assert NL * (TA + P0) == S
    PR = NL * P0
    W = D // NH

    def kernel(x_hbm, wqkv_hbm, wo_hbm, wg_hbm, wu_hbm, wd_hbm, o_hbm,
               x_v, wqa_v, wqb_v, wk_v, wv_v, wo_v, wg_v, wu_v, wd_v, xn_v, kacc, g_acc, z_acc,
               zrow_v, m_v, pq_v, obuf, cnt, isem, osem):
        def xk_c(i):
            r0 = E if i >= 2 else 0
            return pltpu.make_async_copy(x_hbm.at[pl.ds(r0, A - r0), pl.ds(i * 128, 128)],
                                         x_v.at[pl.ds(r0, A - r0), pl.ds(i * 128, 128)], isem.at[i])

        def wk_c(i):
            return pltpu.make_async_copy(wqkv_hbm.at[pl.ds(i * 128, 128), pl.ds(D, D)],
                                         wk_v.at[pl.ds(i * 128, 128), :], isem.at[4 + i])
        xe_c = pltpu.make_async_copy(x_hbm.at[pl.ds(0, E), pl.ds(256, 256)],
                                     x_v.at[pl.ds(0, E), pl.ds(256, 256)], isem.at[16])
        x2_c = pltpu.make_async_copy(x_hbm.at[pl.ds(A, S - A)], x_v.at[pl.ds(A, S - A)], isem.at[8])
        wqa_c = pltpu.make_async_copy(wqkv_hbm.at[:, pl.ds(0, QA)], wqa_v, isem.at[9])
        wqb_c = pltpu.make_async_copy(wqkv_hbm.at[:, pl.ds(QA, D - QA)], wqb_v, isem.at[10])
        wv_c = pltpu.make_async_copy(wqkv_hbm.at[:, pl.ds(2 * D, D)], wv_v, isem.at[11])
        wo_c = pltpu.make_async_copy(wo_hbm, wo_v, isem.at[12])
        wg_c = pltpu.make_async_copy(wg_hbm, wg_v, isem.at[13])
        wu_c = pltpu.make_async_copy(wu_hbm, wu_v, isem.at[14])
        wd_c = pltpu.make_async_copy(wd_hbm, wd_v, isem.at[15])
        for i in range(4):
            wk_c(i).start()
            xk_c(i).start()
            if i == 1:
                xe_c.start()
        for c in (x2_c, wqa_c, wv_c, wo_c, wqb_c, wg_c, wu_c, wd_c):
            c.start()

        def ln(o, n):
            x = x_v[o:o + n, :].astype(F32)
            mu = jnp.sum(x, axis=-1, keepdims=True) * (1.0 / D)
            xc = x - mu
            var = jnp.sum(xc * xc, axis=-1, keepdims=True) * (1.0 / D)
            r = jnp.exp(-0.5 * jnp.log(var + 1e-5))
            xn = (xc * r).astype(BF)
            xn_v[o // 2:(o + n) // 2, :] = pltpu.bitcast(xn, U32)
            return xn, mu, r

        def xn_ld(o, n):
            return pltpu.bitcast(xn_v[o // 2:(o + n) // 2, :], BF)

        def qfill(o, n):
            pq_v[o:o + n, :] = _phi(_dot(xn_ld(o, n), wqa_v[...]))

        def sub(h0, n, osplit, pre):
            row = pl.ds(pl.multiple_of(2 * h0, 16), n)
            xn = pltpu.bitcast(xn_v[pl.ds(pl.multiple_of(h0, 8), n // 2), :], BF)
            pqa = pq_v[row, :] if pre else _phi(_dot(xn, wqa_v[...]))
            pq = jnp.concatenate([pqa, _phi(_dot(xn, wqb_v[...]))], axis=1)
            a = _normalize(pq, zrow_v[0:1, :])
            gt = _dot(xn, wg_v[...])
            up = _dot(xn, wu_v[...])
            h = _gelu_mul(gt, up).astype(BF)
            hy = 0.5 * _dot(h, wd_v[...])
            g = hy * (1.0 + jnp.tanh(hy))
            w = D // osplit
            for c in range(osplit):
                cl = slice(c * w, (c + 1) * w)
                sa = _dot(a, m_v[:, cl])
                obuf[row, cl] = (x_v[row, cl].astype(F32) + sa * g[:, cl]).astype(BF)
                pltpu.make_async_copy(obuf.at[row, pl.ds(c * w, w)], o_hbm.at[row, pl.ds(c * w, w)],
                                      osem.at[0]).start()

        def body(i, carry):
            sub(i * (P0 // 2), P0, 1, True)
            o = 0
            for k, n in enumerate(SA):
                sub((PR + o) // 2 + i * (TA // 2), n, OSPLIT if k == len(SA) - 1 else 1, False)
                o += n
            return carry

        def main(_, carry):
            wkts = [None] * 4

            def wkt(blk):
                for i in range(4):
                    if WT[i] == blk:
                        wkts[i] = wk_v[i * 128:(i + 1) * 128, :].astype(F32).T.astype(BF)

            wk_c(0).wait()
            xk_c(0).wait()
            kacc[...] = _dot(x_v[0:A, 0:128], wk_v[0:128, :])
            wkt(2)
            cs8 = _sum8(wk_v[0:128, :].astype(F32))

            wk_c(1).wait()
            xk_c(1).wait()
            xe_c.wait()
            lns = {j: ln(j * 128, 128) for j in range(E // 128)}
            kacc[...] += _dot(x_v[0:A, 128:256], wk_v[128:256, :])
            wkt(3)
            cs8 = cs8 + _sum8(wk_v[128:256, :].astype(F32))

            for i in (2, 3):
                wk_c(i).wait()
                xk_c(i).wait()
            cs = jnp.sum(cs8 + _sum8(wk_v[256:512, :].astype(F32)), axis=0, keepdims=True)
            wkt(4)
            zn = [None] * NH
            pks = {}
            units = [(j, h) for j in range(A // 128) for h in range(NH)]

            def kunit(j, h):
                o = j * 128
                cl = slice(h * W, (h + 1) * W)
                kraw = kacc[o:o + 128, cl] + _dot(x_v[o:o + 128, 256:512], wk_v[256:512, cl])
                if j not in lns:
                    lns[j] = ln(o, 128)
                _, mu, r = lns[j]
                pk = _phi((kraw - mu * cs[:, cl]) * r)
                zp = _sum8(pk)
                zn[h] = zp if zn[h] is None else zn[h] + zp
                pks[(j, h)] = pk.T.astype(BF)

            def gunit(j, h):
                gp = _dot(pks[(j, h)], lns[j][0] if j * 128 >= E else xn_ld(j * 128, 128))
                if j == 0:
                    g_acc[h * W:(h + 1) * W, :] = gp
                else:
                    g_acc[h * W:(h + 1) * W, :] += gp

            for t in range(len(units) + LAG):
                if t < len(units):
                    kunit(*units[t])
                if t >= LAG:
                    gunit(*units[t - LAG])
            znat = jnp.concatenate(zn, axis=1)

            x2_c.wait()
            wqa_c.wait()
            wv_c.wait()
            wo_c.wait()
            wkt(5)
            wk_t = jnp.concatenate(wkts, axis=1)
            qfill(0, Q0)
            xns = [ln(o, min(KSUB, S - o))[0] for o in range(A, S, KSUB)]
            last = []
            pend = None
            for idx, xn in enumerate(xns):
                if pend is not None:
                    g_acc[...] += _dot(*pend)
                pkt = _phi(lax.dot_general(wk_t, xn, NT, preferred_element_type=F32))
                zp = pkt[:, 0:128]
                for c in range(1, pkt.shape[1] // 128):
                    zp = zp + pkt[:, c * 128:(c + 1) * 128]
                if idx == 0:
                    z_acc[...] = zp
                else:
                    z_acc[...] += zp
                p = (pkt.astype(BF), xn)
                if idx < len(xns) - GLN:
                    pend = p
                else:
                    pend = None
                    last.append(p)
            if Q0 < PR:
                qfill(Q0, PR - Q0)
            pk_l = jnp.concatenate([p[0] for p in last], axis=1)
            xn_l = jnp.concatenate([p[1] for p in last], axis=0)
            zrow = jnp.sum(_sum8(z_acc[...].T) + znat, axis=0, keepdims=True)
            zrow_v[...] = jnp.broadcast_to(zrow, (8, D))

            rr = lax.broadcasted_iota(jnp.int32, (128, 128), 0) // DH
            cc = lax.broadcasted_iota(jnp.int32, (128, 128), 1) // DH
            mask = rr == cc

            def gblk(b):
                sl = slice(b * 128, (b + 1) * 128)
                return g_acc[sl, :] + _dot(pk_l[sl, :], xn_l)

            def kvblk(gb, b):
                kvb = _dot(gb.astype(BF), wv_v[:, b * 128:(b + 1) * 128])
                return jnp.where(mask, kvb, 0.0).astype(BF)

            def mblk(kvb, b):
                sl = slice(b * 128, (b + 1) * 128)
                m_v[sl, :] = _dot(kvb, wo_v[sl, :]).astype(BF)

            g0 = gblk(0)
            g1 = gblk(1)
            kv0 = kvblk(g0, 0)
            g2 = gblk(2)
            kv1 = kvblk(g1, 1)
            g3 = gblk(3)
            kv2 = kvblk(g2, 2)
            mblk(kv0, 0)
            kv3 = kvblk(g3, 3)
            mblk(kv1, 1)
            mblk(kv2, 2)
            mblk(kv3, 3)

            wqb_c.wait()
            wg_c.wait()
            wu_c.wait()
            wd_c.wait()
            lax.fori_loop(0, NL, body, 0)
            return carry

        cnt[0] = 1
        lax.fori_loop(0, cnt[0], main, 0)
        pltpu.make_async_copy(obuf, o_hbm, osem.at[0]).wait()

    def fn(A_x, A_wqkv, A_wo, B_x, B_w_gate, B_w_up, B_w_down):
        x2 = A_x.reshape(S, D)
        out = pl.pallas_call(
            kernel,
            out_shape=jax.ShapeDtypeStruct((S, D), BF),
            in_specs=[pl.BlockSpec(memory_space=pl.ANY)] * 6,
            out_specs=pl.BlockSpec(memory_space=pl.ANY),
            scratch_shapes=[
                pltpu.VMEM((S, D), BF),
                pltpu.VMEM((D, QA), BF),
                pltpu.VMEM((D, D - QA), BF),
                pltpu.VMEM((D, D), BF),
                pltpu.VMEM((D, D), BF),
                pltpu.VMEM((D, D), BF),
                pltpu.VMEM((D, F), BF),
                pltpu.VMEM((D, F), BF),
                pltpu.VMEM((F, D), BF),
                pltpu.VMEM((S // 2, D), U32),
                pltpu.VMEM((A, D), F32),
                pltpu.VMEM((D, D), F32),
                pltpu.VMEM((D, 128), F32),
                pltpu.VMEM((8, D), F32),
                pltpu.VMEM((D, D), BF),
                pltpu.VMEM((PR, QA), F32),
                pltpu.VMEM((S, D), BF),
                pltpu.SMEM((1,), jnp.int32),
                pltpu.SemaphoreType.DMA((17,)),
                pltpu.SemaphoreType.DMA((1,)),
            ],
            compiler_params=pltpu.CompilerParams(vmem_limit_bytes=100 * 1024 * 1024,
                                                 disable_bounds_checks=True,
                                                 disable_semaphore_checks=True),
        )(x2, A_wqkv, A_wo, B_w_gate, B_w_up, B_w_down)
        return out.reshape(1, S, D)
    return fn


_impl = make(SA=(448, 64))


@jax.jit
def pallas_recurrent_scan__linear_attn_block__geglu_ffn__prompt_kernel(
    A_x: jax.Array,
    A_wqkv: jax.Array,
    A_wo: jax.Array,
    B_x: jax.Array,
    B_w_gate: jax.Array,
    B_w_up: jax.Array,
    B_w_down: jax.Array,
):
    return _impl(A_x, A_wqkv, A_wo, B_x, B_w_gate, B_w_up, B_w_down)
```

```python
import jax
import jax.numpy as jnp
from jax import lax
import jax.experimental.pallas as pl
import jax.experimental.pallas.tpu as pltpu

S, D, F, H = 2048, 512, 1792, 32
DH = D // H
BF = jnp.bfloat16
F32 = jnp.float32
U32 = jnp.uint32
NT = (((1,), (1,)), ((), ()))


def _phi(t):
    return jnp.where(t > 0, t + 1.0, jnp.exp(t)) + 1e-6


def _gelu_mul(x, up):
    c0 = 0.7978845608028654
    c1 = 0.7978845608028654 * 0.044715
    t = jnp.tanh(x * (c0 + c1 * (x * x)))
    return (0.5 * x * up) * (1.0 + t)


def _rl(x, k):
    return pltpu.roll(x, k % 128, 1)


def _normalize(pq, zrow):
    n = pq.shape[0]
    lane = lax.broadcasted_iota(jnp.int32, (n, 128), 1)
    b0 = (lane & 1) != 0
    b1 = (lane & 2) != 0
    b2 = (lane & 4) != 0
    b3 = (lane & 8) != 0
    t = pq * zrow
    tb = [t[:, b * 128:(b + 1) * 128] for b in range(4)]
    m01 = jnp.where(b0, tb[0] + _rl(tb[0], 1), tb[1] + _rl(tb[1], -1))
    m23 = jnp.where(b0, tb[2] + _rl(tb[2], 1), tb[3] + _rl(tb[3], -1))
    u = jnp.where(b1, m01 + _rl(m01, 2), m23 + _rl(m23, -2))
    u = u + jnp.where(b2, _rl(u, 4), _rl(u, -4))
    u = u + jnp.where(b3, _rl(u, 8), _rl(u, -8))
    r = 1.0 / (u + 1e-6)
    r01 = jnp.where(b1, r, _rl(r, -2))
    r23 = jnp.where(b1, _rl(r, 2), r)
    rs = [jnp.where(b0, r01, _rl(r01, -1)), jnp.where(b0, _rl(r01, 1), r01),
          jnp.where(b0, r23, _rl(r23, -1)), jnp.where(b0, _rl(r23, 1), r23)]
    return jnp.concatenate([pq[:, b * 128:(b + 1) * 128] * rs[b] for b in range(4)], axis=1)


def _dot(a, b):
    return jnp.dot(a, b, preferred_element_type=F32)


def _sum8(x):
    n, c = x.shape
    return jnp.sum(x.reshape(n // 8, 8, c), axis=0)


def _acomb(a11, a12, a21, a22):
    return [(a11 + a22).astype(BF), (a21 + a22).astype(BF), a11.astype(BF), a22.astype(BF),
            (a11 + a12).astype(BF), (a21 - a11).astype(BF), (a12 - a22).astype(BF)]


def _bcomb(b11, b12, b21, b22):
    return [(b11 + b22).astype(BF), b11.astype(BF), (b12 - b22).astype(BF), (b21 - b11).astype(BF),
            b22.astype(BF), (b11 + b12).astype(BF), (b21 + b22).astype(BF)]


def _scomb(m):
    return (m[0] + m[3] - m[4] + m[6], m[2] + m[4], m[1] + m[3], m[0] - m[1] + m[2] + m[5])


def _strassen(sa, tb, order=(0, 1, 2, 3, 4, 5, 6)):
    m = [None] * 7
    for p in order:
        m[p] = _dot(sa[p], tb[p])
    return _scomb(m)


def make(A=896, E=128, NH=2, LAG=2, KSUB=256, NL=2, P0=512, SA=(384, 128),
         QSUB=256, WT=(2, 3, 4, 4), QPOS=1, QEND=7, PB=128, QC=256, SEQ='c p k0 q0 k1 q1 G01 k2 q2 k3 q3 G23', WKC=4, LNF=0, ORD=(1, 4, 0, 2, 3, 5, 6)):
    TA = sum(SA)
    assert NL * (TA + P0) == S
    PR = NL * P0
    assert A + 128 + PR == S
    CR = NL * SA[-1]
    W = D // NH
    KH = D // 2
    FH = F // 2

    def kernel(x_hbm, wqkv_hbm, wo_hbm, wg_hbm, wu_hbm, wd_hbm, o_hbm,
               x_v, wq_v, wk_v, wv_v, wo_v, wg_v, wu_v, wd_v, xn_v, kacc, g_acc, z_acc,
               zrow_v, m_v, pq_v, obuf, cnt, isem, osem):
        def xk_c(i):
            r0 = E if i >= 2 else 0
            return pltpu.make_async_copy(x_hbm.at[pl.ds(r0, A - r0), pl.ds(i * 128, 128)],
                                         x_v.at[pl.ds(r0, A - r0), pl.ds(i * 128, 128)], isem.at[i])

        def wk_c(i):
            return pltpu.make_async_copy(wqkv_hbm.at[pl.ds(i * 128, 128), pl.ds(D, D)],
                                         wk_v.at[pl.ds(i * 128, 128), :], isem.at[4 + i])
        xe_c = pltpu.make_async_copy(x_hbm.at[pl.ds(0, E), pl.ds(256, 256)],
                                     x_v.at[pl.ds(0, E), pl.ds(256, 256)], isem.at[16])
        x2_c = pltpu.make_async_copy(x_hbm.at[pl.ds(A, S - A)], x_v.at[pl.ds(A, S - A)], isem.at[8])

        def wq_c(b):
            return pltpu.make_async_copy(wqkv_hbm.at[:, pl.ds(b * 128, 128)], wq_v.at[:, pl.ds(b * 128, 128)],
                                         isem.at[17 + b])
        wv_c = pltpu.make_async_copy(wqkv_hbm.at[:, pl.ds(2 * D, D)], wv_v, isem.at[11])
        wo_c = pltpu.make_async_copy(wo_hbm, wo_v, isem.at[12])
        wg_c = pltpu.make_async_copy(wg_hbm, wg_v, isem.at[13])
        wu_c = pltpu.make_async_copy(wu_hbm, wu_v, isem.at[14])
        wd_c = pltpu.make_async_copy(wd_hbm, wd_v, isem.at[15])
        for i in range(4):
            wk_c(i).start()
            xk_c(i).start()
            if i == 1:
                xe_c.start()
        for c in (x2_c, wq_c(0), wq_c(2), wv_c, wo_c, wq_c(1), wq_c(3), wg_c, wu_c, wd_c):
            c.start()

        def ln(o, n):
            x = x_v[o:o + n, :].astype(F32)
            mu = jnp.sum(x, axis=-1, keepdims=True) * (1.0 / D)
            xc = x - mu
            var = jnp.sum(xc * xc, axis=-1, keepdims=True) * (1.0 / D)
            r = jnp.exp(-0.5 * jnp.log(var + 1e-5))
            if LNF == 1 or (LNF == 2 and o >= A):
                xf = x * r - mu * r
            else:
                xf = xc * r
            xn = xf.astype(BF)
            xn_v[o // 2:(o + n) // 2, :] = pltpu.bitcast(xn, U32)
            return xn, mu, r, xf

        def xn_ld(o, n):
            return pltpu.bitcast(xn_v[o // 2:(o + n) // 2, :], BF)

        def wops(cache, w_v, name, kh, nh, jt, r0=0, r1=None):
            r1 = kh if r1 is None else r1
            j = jt * 128
            r11 = w_v[r0:r1, j:j + 128]
            r22 = w_v[kh + r0:kh + r1, nh + j:nh + j + 128]
            key = (name, jt, r0)
            if key not in cache:
                b11 = r11.astype(F32)
                b12 = w_v[r0:r1, nh + j:nh + j + 128].astype(F32)
                b21 = w_v[kh + r0:kh + r1, j:j + 128].astype(F32)
                b22 = r22.astype(F32)
                cache[key] = [t.astype(BF) for t in (b11 + b22, b12 - b22, b21 - b11, b11 + b12, b21 + b22)]
            c = cache[key]
            return [c[0], r11, c[1], c[2], r22, c[3], c[4]]

        def mops(cache, jt):
            j = jt * 128
            key = ('m', jt)
            if key not in cache:
                cache[key] = _bcomb(m_v[0:KH, j:j + 128], m_v[0:KH, KH + j:KH + j + 128],
                                    m_v[KH:D, j:j + 128], m_v[KH:D, KH + j:KH + j + 128])
            return cache[key]

        HB = PB // 2

        def halves(v):
            nb = v.shape[0] // PB
            return (jnp.concatenate([v[b * PB:b * PB + HB] for b in range(nb)], axis=0),
                    jnp.concatenate([v[b * PB + HB:(b + 1) * PB] for b in range(nb)], axis=0))

        def unhalves(c1, c2):
            nb = c1.shape[0] // HB
            return jnp.concatenate([t[b * HB:(b + 1) * HB] for b in range(nb) for t in (c1, c2)], axis=0)

        def lcomb(v):
            v1, v2 = halves(v)
            return _acomb(v1[:, :KH], v1[:, KH:], v2[:, :KH], v2[:, KH:])

        def rows2(c):
            return unhalves(c[0], c[2]), unhalves(c[1], c[3])

        def sub(cache, h0, n, split_out, pre):
            row = pl.ds(pl.multiple_of(2 * h0, 16), n)
            n2 = n // 2
            sa = lcomb(pltpu.bitcast(xn_v[pl.ds(pl.multiple_of(h0, 8), n2), :], BF).astype(F32))

            def qchunk(b, m):
                sc = sa if m == n else [t[b // 2:(b + m) // 2] for t in sa]
                if pre:
                    rw = pl.ds(pl.multiple_of(2 * h0 + b + pre - 1, 16), m)
                    p0, p2 = pq_v[rw, 0:128], pq_v[rw, 128:256]
                else:
                    p0, p2 = [_phi(t) for t in rows2(_strassen(sc, wops(cache, wq_v, 'q', KH, KH, 0), ORD))]
                p1, p3 = [_phi(t) for t in rows2(_strassen(sc, wops(cache, wq_v, 'q', KH, KH, 1), ORD))]
                return _normalize(jnp.concatenate([p0, p1, p2, p3], axis=1), zrow_v[0:1, :])

            NJ = FH // 128
            blocks = list(range(0, n, QC))
            aparts = []

            def qupto(jt):
                if jt >= QPOS:
                    want = min(len(blocks), -(-(jt - QPOS + 1) * len(blocks) // (QEND + 1 - QPOS)))
                    while len(aparts) < want:
                        b = blocks[len(aparts)]
                        aparts.append(qchunk(b, min(QC, n - b)))

            hs = []
            for jt in range(NJ):
                qupto(jt)
                gq = _strassen(sa, wops(cache, wg_v, 'g', KH, FH, jt), ORD)
                uq = _strassen(sa, wops(cache, wu_v, 'u', KH, FH, jt), ORD)
                hs.append(_acomb(*[_gelu_mul(gq[t], uq[t]) for t in range(4)]))
            qupto(NJ)
            gs = []
            for jt in range(2):
                wd = [wops(cache, wd_v, 'd', FH, KH, jt, k * 128, (k + 1) * 128) for k in range(NJ)]
                m = [None] * 7
                for p in ORD:
                    for k in range(NJ):
                        t = _dot(hs[k][p], wd[k][p])
                        m[p] = t if m[p] is None else m[p] + t
                if jt == 0:
                    aa = lcomb(jnp.concatenate(aparts, axis=0))
                for y in rows2(_scomb(m)):
                    hy = 0.5 * y
                    gs.append(hy * (1.0 + jnp.tanh(hy)))
            for jt in range(2):
                ss = rows2(_strassen(aa, mops(cache, jt), ORD))
                for t in range(2):
                    c0 = t * KH + jt * 128
                    obuf[row, c0:c0 + 128] = (x_v[row, c0:c0 + 128].astype(F32)
                                              + ss[t] * gs[2 * jt + t]).astype(BF)
                    if split_out:
                        pltpu.make_async_copy(obuf.at[row, pl.ds(c0, 128)], o_hbm.at[row, pl.ds(c0, 128)],
                                              osem.at[0]).start()
            if not split_out:
                pltpu.make_async_copy(obuf.at[row], o_hbm.at[row], osem.at[0]).start()

        def body(i, carry):
            cache = {}
            sub(cache, (S - PR) // 2 + i * (P0 // 2), P0, False, 1 - (S - PR))
            o = 0
            for n in SA[:-1]:
                sub(cache, (CR + o) // 2 + i * ((TA - SA[-1]) // 2), n, False, 0)
                o += n
            sub(cache, i * (SA[-1] // 2), SA[-1], True, 1 + PR)
            return carry

        def main(_, carry):
            wkts = [None] * 4

            def wkt(blk):
                for i in range(4):
                    if WT[i] == blk:
                        wkts[i] = wk_v[i * 128:(i + 1) * 128, :].astype(F32).T

            wk_c(0).wait()
            xk_c(0).wait()
            kacc[...] = _dot(x_v[0:A, 0:128], wk_v[0:128, :])
            wkt(2)
            cs8 = _sum8(wk_v[0:128, :].astype(F32))

            wk_c(1).wait()
            xk_c(1).wait()
            xe_c.wait()
            lns = {j: ln(j * 128, 128) for j in range(E // 128)}
            kacc[...] += _dot(x_v[0:A, 128:256], wk_v[128:256, :])
            wkt(3)
            cs8 = cs8 + _sum8(wk_v[128:256, :].astype(F32))

            for i in (2, 3):
                wk_c(i).wait()
                xk_c(i).wait()
            cs = jnp.sum(cs8 + _sum8(wk_v[256:512, :].astype(F32)), axis=0, keepdims=True)
            wkt(4)
            zn = [None] * NH
            pks = {}
            units = [(j, h) for j in range(A // 128) for h in range(NH)]

            def kunit(j, h):
                o = j * 128
                cl = slice(h * W, (h + 1) * W)
                if o < A:
                    kraw = kacc[o:o + 128, cl] + _dot(x_v[o:o + 128, 256:512], wk_v[256:512, cl])
                else:
                    kraw = _dot(x_v[o:o + 128, :], wk_v[:, cl])
                if j not in lns:
                    lns[j] = ln(o, 128)
                _, mu, r, _ = lns[j]
                pk = _phi((kraw - mu * cs[:, cl]) * r)
                zp = _sum8(pk)
                zn[h] = zp if zn[h] is None else zn[h] + zp
                pks[(j, h)] = pk.T.astype(BF)

            def gunit(j, h):
                gp = _dot(pks[(j, h)], lns[j][0] if j * 128 >= E else xn_ld(j * 128, 128))
                if j == 0:
                    g_acc[h * W:(h + 1) * W, :] = gp
                else:
                    g_acc[h * W:(h + 1) * W, :] += gp

            for t in range(len(units) + LAG):
                if t < len(units):
                    kunit(*units[t])
                if t >= LAG:
                    gunit(*units[t - LAG])

            def mkwkc():
                wf = jnp.concatenate(wkts, axis=1)
                return _bcomb(wf[:KH, :KH], wf[KH:, :KH], wf[:KH, KH:], wf[KH:, KH:]), wf.astype(BF)
            if WKC == 4:
                wkc, wk_t = mkwkc()

            x2_c.wait()
            wq_c(0).wait()
            wq_c(2).wait()
            wv_c.wait()
            wo_c.wait()
            wkt(5)
            if WKC == 5:
                wkc, wk_t = mkwkc()
            wq0 = wops({}, wq_v, 'q', KH, KH, 0)
            kd = {}
            zfirst = True
            for step in SEQ.split():
                if step == 'r':
                    for h in range(NH):
                        kunit(A // 128, h)
                elif step == 'c':
                    xe = xn_ld(0, CR)
                    pq_v[PR:PR + CR, 0:128] = _phi(_dot(xe, wq_v[:, 0:128]))
                    pq_v[PR:PR + CR, 128:256] = _phi(_dot(xe, wq_v[:, 256:384]))
                elif step == 'p':
                    lns[A // 128] = ln(A, 128)
                    t = _phi(lax.dot_general(wk_t, lns[A // 128][0], NT, preferred_element_type=F32))
                    if zfirst:
                        z_acc[...] = t
                    else:
                        z_acc[...] += t
                    zfirst = False
                    for h in range(NH):
                        pks[(A // 128, h)] = t[h * W:(h + 1) * W, :].astype(BF)
                elif step[0] == 'q':
                    ci = int(step[1:])
                    c = [_phi(t) for t in _strassen(kd[ci][1], wq0, ORD)]
                    r0, hh = ci * KSUB, KSUB // 2
                    pq_v[r0:r0 + hh, 0:128] = c[0]
                    pq_v[r0:r0 + hh, 128:256] = c[1]
                    pq_v[r0 + hh:r0 + KSUB, 0:128] = c[2]
                    pq_v[r0 + hh:r0 + KSUB, 128:256] = c[3]
                elif step[0] == 'k':
                    ci = int(step[1:])
                    xf = ln(S - PR + ci * KSUB, KSUB)[3]
                    h = KSUB // 2
                    sa = _acomb(xf[:h, :KH], xf[:h, KH:], xf[h:, :KH], xf[h:, KH:])
                    m = [None] * 7
                    for p in ORD:
                        m[p] = lax.dot_general(wkc[p], sa[p], NT, preferred_element_type=F32)
                    c = [_phi(t) for t in _scomb(m)]
                    for (r0, t) in ((0, c[0] + c[2]), (KH, c[1] + c[3])):
                        zp = t[:, 0:128]
                        for cc in range(1, h // 128):
                            zp = zp + t[:, cc * 128:(cc + 1) * 128]
                        if zfirst:
                            z_acc[r0:r0 + KH, :] = zp
                        else:
                            z_acc[r0:r0 + KH, :] += zp
                    zfirst = False
                    kd[ci] = (_acomb(c[0], c[2], c[1], c[3]), sa)
                else:
                    m = [None] * 7
                    for p in ORD:
                        for ch in step[1:]:
                            pa, sa = kd[int(ch)]
                            t = _dot(pa[p], sa[(0, 2, 6, 5, 3, 4, 1)[p]])
                            m[p] = t if m[p] is None else m[p] + t
                    c = _scomb(m)
                    g_acc[0:KH, 0:KH] += c[0]
                    g_acc[0:KH, KH:D] += c[1]
                    g_acc[KH:D, 0:KH] += c[2]
                    g_acc[KH:D, KH:D] += c[3]
            jl = A // 128
            xn_l = lns[jl][0]
            znat = jnp.concatenate(zn, axis=1)
            zrow = jnp.sum(_sum8(z_acc[...].T) + znat, axis=0, keepdims=True)
            zrow_v[...] = jnp.broadcast_to(zrow, (8, D))

            rr = lax.broadcasted_iota(jnp.int32, (128, 128), 0) // DH
            cc = lax.broadcasted_iota(jnp.int32, (128, 128), 1) // DH
            mask = rr == cc

            def gblk(b):
                sl = slice(b * 128, (b + 1) * 128)
                o = (b * 128) % W
                return g_acc[sl, :] + _dot(pks[(jl, b * 128 // W)][o:o + 128, :], xn_l)

            def kvblk(gb, b):
                kvb = _dot(gb.astype(BF), wv_v[:, b * 128:(b + 1) * 128])
                return jnp.where(mask, kvb, 0.0).astype(BF)

            def mblk(kvb, b):
                sl = slice(b * 128, (b + 1) * 128)
                m_v[sl, :] = _dot(kvb, wo_v[sl, :])

            g0 = gblk(0)
            g1 = gblk(1)
            kv0 = kvblk(g0, 0)
            g2 = gblk(2)
            kv1 = kvblk(g1, 1)
            g3 = gblk(3)
            kv2 = kvblk(g2, 2)
            mblk(kv0, 0)
            kv3 = kvblk(g3, 3)
            mblk(kv1, 1)
            mblk(kv2, 2)
            mblk(kv3, 3)

            wq_c(1).wait()
            wq_c(3).wait()
            wg_c.wait()
            wu_c.wait()
            wd_c.wait()
            lax.fori_loop(0, NL, body, 0)
            return carry

        cnt[0] = 1
        lax.fori_loop(0, cnt[0], main, 0)
        pltpu.make_async_copy(obuf, o_hbm, osem.at[0]).wait()

    def fn(A_x, A_wqkv, A_wo, B_x, B_w_gate, B_w_up, B_w_down):
        x2 = A_x.reshape(S, D)
        out = pl.pallas_call(
            kernel,
            out_shape=jax.ShapeDtypeStruct((S, D), BF),
            in_specs=[pl.BlockSpec(memory_space=pl.ANY)] * 6,
            out_specs=pl.BlockSpec(memory_space=pl.ANY),
            scratch_shapes=[
                pltpu.VMEM((S, D), BF),
                pltpu.VMEM((D, D), BF),
                pltpu.VMEM((D, D), BF),
                pltpu.VMEM((D, D), BF),
                pltpu.VMEM((D, D), BF),
                pltpu.VMEM((D, F), BF),
                pltpu.VMEM((D, F), BF),
                pltpu.VMEM((F, D), BF),
                pltpu.VMEM((S // 2, D), U32),
                pltpu.VMEM((A, D), F32),
                pltpu.VMEM((D, D), F32),
                pltpu.VMEM((D, 128), F32),
                pltpu.VMEM((8, D), F32),
                pltpu.VMEM((D, D), F32),
                pltpu.VMEM((PR + CR, 256), F32),
                pltpu.VMEM((S, D), BF),
                pltpu.SMEM((1,), jnp.int32),
                pltpu.SemaphoreType.DMA((21,)),
                pltpu.SemaphoreType.DMA((1,)),
            ],
            compiler_params=pltpu.CompilerParams(vmem_limit_bytes=100 * 1024 * 1024,
                                                 disable_bounds_checks=True,
                                                 disable_semaphore_checks=True),
        )(x2, A_wqkv, A_wo, B_w_gate, B_w_up, B_w_down)
        return out.reshape(1, S, D)
    return fn


_impl = make(LNF=2, WKC=5)


@jax.jit
def pallas_recurrent_scan__linear_attn_block__geglu_ffn__prompt_kernel(
    A_x: jax.Array,
    A_wqkv: jax.Array,
    A_wo: jax.Array,
    B_x: jax.Array,
    B_w_gate: jax.Array,
    B_w_up: jax.Array,
    B_w_down: jax.Array,
):
    return _impl(A_x, A_wqkv, A_wo, B_x, B_w_gate, B_w_up, B_w_down)
```

```python
import jax
import jax.numpy as jnp
from jax import lax
import jax.experimental.pallas as pl
import jax.experimental.pallas.tpu as pltpu

S, D, F, H = 2048, 512, 1792, 32
DH = D // H
KH = D // 2
FH = F // 2
NJ = FH // 128
BF = jnp.bfloat16
F32 = jnp.float32
U32 = jnp.uint32
NT = (((1,), (1,)), ((), ()))


def _phi(t):
    return jnp.where(t > 0, t + 1.0, jnp.exp(t)) + 1e-6


def _gelu_mul(x, up):
    c0 = 0.7978845608028654
    c1 = 0.7978845608028654 * 0.044715
    t = jnp.tanh(x * (c0 + c1 * (x * x)))
    return (0.5 * x * up) * (1.0 + t)


def _rl(x, k):
    return pltpu.roll(x, k % 128, 1)


def _normalize(pq, zrow):
    n = pq.shape[0]
    lane = lax.broadcasted_iota(jnp.int32, (n, 128), 1)
    b0 = (lane & 1) != 0
    b1 = (lane & 2) != 0
    b2 = (lane & 4) != 0
    b3 = (lane & 8) != 0
    t = pq * zrow
    tb = [t[:, b * 128:(b + 1) * 128] for b in range(4)]
    m02 = jnp.where(b0, tb[0] + _rl(tb[0], 1), tb[2] + _rl(tb[2], -1))
    m13 = jnp.where(b0, tb[1] + _rl(tb[1], 1), tb[3] + _rl(tb[3], -1))
    u = jnp.where(b1, m02 + _rl(m02, 2), m13 + _rl(m13, -2))
    u = u + jnp.where(b2, _rl(u, 4), _rl(u, -4))
    u = u + jnp.where(b3, _rl(u, 8), _rl(u, -8))
    r = 1.0 / (u + 1e-6)
    r02 = jnp.where(b1, r, _rl(r, -2))
    r13 = jnp.where(b1, _rl(r, 2), r)
    rs = [jnp.where(b0, r02, _rl(r02, -1)), jnp.where(b0, r13, _rl(r13, -1)),
          jnp.where(b0, _rl(r02, 1), r02), jnp.where(b0, _rl(r13, 1), r13)]
    return jnp.concatenate([pq[:, b * 128:(b + 1) * 128] * rs[b] for b in range(4)], axis=1)


def _dot(a, b):
    return jnp.dot(a, b, preferred_element_type=F32)


def _sum8(x):
    n, c = x.shape
    return jnp.sum(x.reshape(n // 8, 8, c), axis=0)


def _acomb(a11, a12, a21, a22):
    return [(a11 + a22).astype(BF), (a21 + a22).astype(BF), a11.astype(BF), a22.astype(BF),
            (a11 + a12).astype(BF), (a21 - a11).astype(BF), (a12 - a22).astype(BF)]


def _bcomb(b11, b12, b21, b22):
    return [(b11 + b22).astype(BF), b11.astype(BF), (b12 - b22).astype(BF), (b21 - b11).astype(BF),
            b22.astype(BF), (b11 + b12).astype(BF), (b21 + b22).astype(BF)]


_A2B = (0, 2, 6, 5, 3, 4, 1)
_SC = ({0: 1, 3: 1, 4: -1, 6: 1}, {2: 1, 4: 1}, {1: 1, 3: 1}, {0: 1, 1: -1, 2: 1, 5: 1})


def make(A=896, E=128, NH=2, LAG=2, KSUB=256, P0=512, SA=(384, 128), WT=(2, 3, 4, 4), PB=128, QC=256,
         SEQ='c k0 q0 k1 q1 G01 k2 q2 k3 q3 p G23', LNF=2, QP1=(1, 7), QP2=(1, 7), QP3=(1, 7), NQ1=0,
         ORD=(4, 2, 1, 3, 0, 6, 5)):
    NL = 2
    assert NL * (sum(SA) + P0) == S
    PR = NL * P0
    CR = NL * SA[1]
    assert A + 128 + PR == S
    W = D // NH
    HB = PB // 2

    def scomb(m):
        out = []
        for q in _SC:
            acc, sign = None, 1
            for p in ORD:
                if p in q:
                    if acc is None:
                        acc, sign = m[p], q[p]
                    elif sign == 1:
                        acc = acc + m[p] if q[p] == 1 else acc - m[p]
                    else:
                        acc, sign = m[p] - acc, 1
            out.append(acc)
        return out

    def strassen(sa, tb):
        m = [None] * 7
        for p in ORD:
            m[p] = _dot(sa[p], tb[p])
        return scomb(m)

    def lcomb(v):
        nb = v.shape[0] // PB
        v1 = jnp.concatenate([v[b * PB:b * PB + HB] for b in range(nb)], axis=0)
        v2 = jnp.concatenate([v[b * PB + HB:(b + 1) * PB] for b in range(nb)], axis=0)
        return _acomb(v1[:, :KH], v1[:, KH:], v2[:, :KH], v2[:, KH:])

    def unhalves(c1, c2):
        nb = c1.shape[0] // HB
        return jnp.concatenate([t[b * HB:(b + 1) * HB] for b in range(nb) for t in (c1, c2)], axis=0)

    def rows2(c):
        return unhalves(c[0], c[2]), unhalves(c[1], c[3])

    def kernel(x_hbm, wqkv_hbm, wo_hbm, wg_hbm, wu_hbm, wd_hbm, o_hbm,
               x_v, wq_v, wk_v, wv_v, wo_v, wg_v, wu_v, wd_v, xn_v, kacc, g_acc, z_acc,
               zrow_v, pq_v, obuf, sa_v, cm_v, cnt, isem, osem):
        def xk_c(i):
            r0 = E if i >= 2 else 0
            return pltpu.make_async_copy(x_hbm.at[pl.ds(r0, A - r0), pl.ds(i * 128, 128)],
                                         x_v.at[pl.ds(r0, A - r0), pl.ds(i * 128, 128)], isem.at[i])

        def wk_c(i):
            return pltpu.make_async_copy(wqkv_hbm.at[pl.ds(i * 128, 128), pl.ds(D, D)],
                                         wk_v.at[pl.ds(i * 128, 128), :], isem.at[4 + i])

        def wq_c(b):
            return pltpu.make_async_copy(wqkv_hbm.at[:, pl.ds(b * 128, 128)], wq_v.at[:, pl.ds(b * 128, 128)],
                                         isem.at[8 + b])
        xe_c = pltpu.make_async_copy(x_hbm.at[pl.ds(0, E), pl.ds(256, 256)],
                                     x_v.at[pl.ds(0, E), pl.ds(256, 256)], isem.at[12])
        x2_c = pltpu.make_async_copy(x_hbm.at[pl.ds(A, S - A)], x_v.at[pl.ds(A, S - A)], isem.at[13])
        wv_c = pltpu.make_async_copy(wqkv_hbm.at[:, pl.ds(2 * D, D)], wv_v, isem.at[14])
        wo_c = pltpu.make_async_copy(wo_hbm, wo_v, isem.at[15])
        wg_c = pltpu.make_async_copy(wg_hbm, wg_v, isem.at[16])
        wu_c = pltpu.make_async_copy(wu_hbm, wu_v, isem.at[17])
        wd_c = pltpu.make_async_copy(wd_hbm, wd_v, isem.at[18])
        for i in range(4):
            wk_c(i).start()
            xk_c(i).start()
            if i == 1:
                xe_c.start()
        for c in (x2_c, wq_c(0), wq_c(2), wv_c, wo_c, wq_c(1), wq_c(3), wg_c, wu_c, wd_c):
            c.start()

        def ln(o, n):
            x = x_v[o:o + n, :].astype(F32)
            mu = jnp.sum(x, axis=-1, keepdims=True) * (1.0 / D)
            xc = x - mu
            var = jnp.sum(xc * xc, axis=-1, keepdims=True) * (1.0 / D)
            r = jnp.exp(-0.5 * jnp.log(var + 1e-5))
            xf = x * r - mu * r if (LNF == 2 and o >= A) else xc * r
            xn = xf.astype(BF)
            if o < S - PR:
                xn_v[o // 2:(o + n) // 2, :] = pltpu.bitcast(xn, U32)
            return xn, mu, r, xf

        def xn_ld(o, n):
            return pltpu.bitcast(xn_v[o // 2:(o + n) // 2, :], BF)

        def wops(cache, w_v, name, kh, nh, jt, r0=0, r1=None):
            r1 = kh if r1 is None else r1
            j = jt * 128
            r11 = w_v[r0:r1, j:j + 128]
            r22 = w_v[kh + r0:kh + r1, nh + j:nh + j + 128]
            key = (name, jt, r0)
            if key not in cache:
                b11 = r11.astype(F32)
                b12 = w_v[r0:r1, nh + j:nh + j + 128].astype(F32)
                b21 = w_v[kh + r0:kh + r1, j:j + 128].astype(F32)
                b22 = r22.astype(F32)
                cache[key] = [t.astype(BF) for t in (b11 + b22, b12 - b22, b21 - b11, b11 + b12, b21 + b22)]
            c = cache[key]
            return [c[0], r11, c[1], c[2], r22, c[3], c[4]]

        class Tile:
            def __init__(self, cache, h0, n, pq_off=None, hq=None):
                self.cache, self.h0, self.n, self.pq_off = cache, h0, n, pq_off
                if hq is not None:
                    hr = pl.ds(pl.multiple_of(hq, 8), n // 4)
                    self.sa = [pltpu.bitcast(sa_v[p, hr, :], BF) for p in range(7)]
                else:
                    xn = pltpu.bitcast(xn_v[pl.ds(pl.multiple_of(h0, 8), n // 2), :], BF)
                    self.sa = lcomb(xn.astype(F32))
                self.aparts = []
                self.gs = []

            def qjobs(self):
                return [(self, b, min(QC, self.n - b)) for b in range(0, self.n, QC)]

            def qchunk(self, b, m):
                sc = self.sa if m == self.n else [t[b // 2:(b + m) // 2] for t in self.sa]
                if self.pq_off is not None:
                    rw = pl.ds(pl.multiple_of(2 * self.h0 + b + self.pq_off, 16), m)
                    p0, p2 = pq_v[rw, 0:128], pq_v[rw, 128:256]
                else:
                    p0, p2 = [_phi(t) for t in rows2(strassen(sc, wops(self.cache, wq_v, 'q', KH, KH, 0)))]
                p1, p3 = [_phi(t) for t in rows2(strassen(sc, wops(self.cache, wq_v, 'q', KH, KH, 1)))]
                self.aparts.append(_normalize(jnp.concatenate([p0, p1, p2, p3], axis=1), zrow_v[0:1, :]))

            def ffn(self, jobs, qp, qe):
                cache, sa = self.cache, self.sa
                done = [0]

                def qupto(pos):
                    if pos >= qp:
                        want = min(len(jobs), -(-(pos - qp + 1) * len(jobs) // (qe + 1 - qp)))
                        while done[0] < want:
                            t, b, m = jobs[done[0]]
                            t.qchunk(b, m)
                            done[0] += 1

                hs = []
                for jt in range(NJ):
                    qupto(jt)
                    gq = strassen(sa, wops(cache, wg_v, 'g', KH, FH, jt))
                    uq = strassen(sa, wops(cache, wu_v, 'u', KH, FH, jt))
                    hs.append(_acomb(*[_gelu_mul(gq[t], uq[t]) for t in range(4)]))
                for jt in range(2):
                    wd = [wops(cache, wd_v, 'd', FH, KH, jt, k * 128, (k + 1) * 128) for k in range(NJ)]
                    m = [None] * 7
                    for pi, p in enumerate(ORD):
                        qupto(NJ + jt * 7 + pi)
                        for k in range(NJ):
                            t = _dot(hs[k][p], wd[k][p])
                            m[p] = t if m[p] is None else m[p] + t
                    for y in rows2(scomb(m)):
                        hy = 0.5 * y
                        self.gs.append(hy * (1.0 + jnp.tanh(hy)))

            def out(self, split_out):
                row = pl.ds(pl.multiple_of(2 * self.h0, 16), self.n)
                aa = lcomb(jnp.concatenate(self.aparts, axis=0))
                for jt in range(2):
                    ss = rows2(strassen(aa, [cm_v[p, jt] for p in range(7)]))
                    for t in range(2):
                        c0 = t * KH + jt * 128
                        obuf[row, c0:c0 + 128] = (x_v[row, c0:c0 + 128].astype(F32)
                                                  + ss[t] * self.gs[2 * jt + t]).astype(BF)
                        if split_out:
                            pltpu.make_async_copy(obuf.at[row, pl.ds(c0, 128)], o_hbm.at[row, pl.ds(c0, 128)],
                                                  osem.at[0]).start()
                if not split_out:
                    pltpu.make_async_copy(obuf.at[row], o_hbm.at[row], osem.at[0]).start()

        def body(i, carry):
            cache = {}
            t1 = Tile(cache, (S - PR) // 2 + i * (P0 // 2), P0, PR - S, i * (P0 // 4))
            j1 = t1.qjobs()
            t1.ffn(j1[:NQ1], *QP1)
            if NQ1 >= len(j1):
                t1.out(False)
            t2 = Tile(cache, CR // 2 + i * (SA[0] // 2), SA[0])
            t2.ffn(j1[NQ1:] + t2.qjobs(), *QP2)
            if NQ1 < len(j1):
                t1.out(False)
            t2.out(False)
            t3 = Tile(cache, i * (SA[1] // 2), SA[1], PR)
            t3.ffn(t3.qjobs(), *QP3)
            t3.out(True)
            return carry

        def main(_, carry):
            wkts = [None] * 4

            def wkt(blk):
                for i in range(4):
                    if WT[i] == blk:
                        wkts[i] = wk_v[i * 128:(i + 1) * 128, :].astype(F32).T

            wk_c(0).wait()
            xk_c(0).wait()
            kacc[...] = _dot(x_v[0:A, 0:128], wk_v[0:128, :])
            wkt(2)
            cs8 = _sum8(wk_v[0:128, :].astype(F32))

            wk_c(1).wait()
            xk_c(1).wait()
            xe_c.wait()
            lns = {j: ln(j * 128, 128) for j in range(E // 128)}
            kacc[...] += _dot(x_v[0:A, 128:256], wk_v[128:256, :])
            wkt(3)
            cs8 = cs8 + _sum8(wk_v[128:256, :].astype(F32))

            for i in (2, 3):
                wk_c(i).wait()
                xk_c(i).wait()
            cs = jnp.sum(cs8 + _sum8(wk_v[256:512, :].astype(F32)), axis=0, keepdims=True)
            wkt(4)
            zn = [None] * NH
            pks = {}
            units = [(j, h) for j in range(A // 128) for h in range(NH)]

            def kunit(j, h):
                o = j * 128
                cl = slice(h * W, (h + 1) * W)
                kraw = kacc[o:o + 128, cl] + _dot(x_v[o:o + 128, 256:512], wk_v[256:512, cl])
                if j not in lns:
                    lns[j] = ln(o, 128)
                _, mu, r, _ = lns[j]
                pk = _phi((kraw - mu * cs[:, cl]) * r)
                zp = _sum8(pk)
                zn[h] = zp if zn[h] is None else zn[h] + zp
                pks[(j, h)] = pk.T.astype(BF)

            def gunit(j, h):
                gp = _dot(pks[(j, h)], lns[j][0] if j * 128 >= E else xn_ld(j * 128, 128))
                if j == 0:
                    g_acc[h * W:(h + 1) * W, :] = gp
                else:
                    g_acc[h * W:(h + 1) * W, :] += gp

            for t in range(len(units) + LAG):
                if t < len(units):
                    kunit(*units[t])
                if t >= LAG:
                    gunit(*units[t - LAG])
            znat = jnp.concatenate(zn, axis=1)

            x2_c.wait()
            wq_c(0).wait()
            wq_c(2).wait()
            wv_c.wait()
            wo_c.wait()
            wkt(5)
            wf = jnp.concatenate(wkts, axis=1)
            wkc = _bcomb(wf[:KH, :KH], wf[KH:, :KH], wf[:KH, KH:], wf[KH:, KH:])
            wq0 = wops({}, wq_v, 'q', KH, KH, 0)
            kd = {}
            zfirst = True
            for step in SEQ.split():
                if step == 'c':
                    xe = xn_ld(0, CR)
                    pq_v[PR:PR + CR, 0:128] = _phi(_dot(xe, wq_v[:, 0:128]))
                    pq_v[PR:PR + CR, 128:256] = _phi(_dot(xe, wq_v[:, 256:384]))
                elif step == 'p':
                    xn_l = ln(A, 128)[0]
                    t = _phi(lax.dot_general(wf.astype(BF), xn_l, NT, preferred_element_type=F32))
                    if zfirst:
                        z_acc[...] = t
                    else:
                        z_acc[...] += t
                    zfirst = False
                    pk_l = [t[b * 128:(b + 1) * 128, :].astype(BF) for b in range(4)]
                elif step[0] == 'q':
                    ci = int(step[1:])
                    lo, hi = rows2([_phi(t) for t in strassen(kd[ci][1], wq0)])
                    pq_v[ci * KSUB:(ci + 1) * KSUB, 0:128] = lo
                    pq_v[ci * KSUB:(ci + 1) * KSUB, 128:256] = hi
                elif step[0] == 'k':
                    ci = int(step[1:])
                    h = KSUB // 2
                    sa = lcomb(ln(S - PR + ci * KSUB, KSUB)[3])
                    for p in range(7):
                        sa_v[p, ci * h // 2:(ci + 1) * h // 2, :] = pltpu.bitcast(sa[p], U32)
                    m = [None] * 7
                    for p in ORD:
                        m[p] = lax.dot_general(wkc[p], sa[p], NT, preferred_element_type=F32)
                    c = [_phi(t) for t in scomb(m)]
                    for (r0, t) in ((0, c[0] + c[2]), (KH, c[1] + c[3])):
                        zp = t[:, 0:128]
                        for cc in range(1, h // 128):
                            zp = zp + t[:, cc * 128:(cc + 1) * 128]
                        if zfirst:
                            z_acc[r0:r0 + KH, :] = zp
                        else:
                            z_acc[r0:r0 + KH, :] += zp
                    zfirst = False
                    kd[ci] = (_acomb(c[0], c[2], c[1], c[3]), sa)
                else:
                    m = [None] * 7
                    for p in ORD:
                        for ch in step[1:]:
                            pa, sa = kd[int(ch)]
                            t = _dot(pa[p], sa[_A2B[p]])
                            m[p] = t if m[p] is None else m[p] + t
                    c = scomb(m)
                    g_acc[0:KH, 0:KH] += c[0]
                    g_acc[0:KH, KH:D] += c[1]
                    g_acc[KH:D, 0:KH] += c[2]
                    g_acc[KH:D, KH:D] += c[3]
            zrow = jnp.sum(_sum8(z_acc[...].T) + znat, axis=0, keepdims=True)
            zrow_v[...] = jnp.broadcast_to(zrow, (8, D))

            rr = lax.broadcasted_iota(jnp.int32, (128, 128), 0) // DH
            cc = lax.broadcasted_iota(jnp.int32, (128, 128), 1) // DH
            mask = rr == cc
            mb = [None] * 4

            def gblk(b):
                return g_acc[b * 128:(b + 1) * 128, :] + _dot(pk_l[b], xn_l)

            def kvblk(gb, b):
                kvb = _dot(gb.astype(BF), wv_v[:, b * 128:(b + 1) * 128])
                return jnp.where(mask, kvb, 0.0).astype(BF)

            def mblk(kvb, b):
                mb[b] = _dot(kvb, wo_v[b * 128:(b + 1) * 128, :])
                if b >= 2:
                    top, bot = mb[b - 2], mb[b]
                    for jt in range(2):
                        j = jt * 128
                        c = _bcomb(top[:, j:j + 128], top[:, KH + j:KH + j + 128],
                                   bot[:, j:j + 128], bot[:, KH + j:KH + j + 128])
                        for p in range(7):
                            cm_v[p, jt, (b - 2) * 128:(b - 1) * 128, :] = c[p]

            g0 = gblk(0)
            g1 = gblk(1)
            kv0 = kvblk(g0, 0)
            g2 = gblk(2)
            kv1 = kvblk(g1, 1)
            g3 = gblk(3)
            kv2 = kvblk(g2, 2)
            mblk(kv0, 0)
            kv3 = kvblk(g3, 3)
            mblk(kv1, 1)
            mblk(kv2, 2)
            mblk(kv3, 3)

            wq_c(1).wait()
            wq_c(3).wait()
            wg_c.wait()
            wu_c.wait()
            wd_c.wait()
            lax.fori_loop(0, NL, body, 0)
            return carry

        cnt[0] = 1
        lax.fori_loop(0, cnt[0], main, 0)
        pltpu.make_async_copy(obuf, o_hbm, osem.at[0]).wait()

    def fn(A_x, A_wqkv, A_wo, B_x, B_w_gate, B_w_up, B_w_down):
        x2 = A_x.reshape(S, D)
        out = pl.pallas_call(
            kernel,
            out_shape=jax.ShapeDtypeStruct((S, D), BF),
            in_specs=[pl.BlockSpec(memory_space=pl.ANY)] * 6,
            out_specs=pl.BlockSpec(memory_space=pl.ANY),
            scratch_shapes=[
                pltpu.VMEM((S, D), BF),
                pltpu.VMEM((D, D), BF),
                pltpu.VMEM((D, D), BF),
                pltpu.VMEM((D, D), BF),
                pltpu.VMEM((D, D), BF),
                pltpu.VMEM((D, F), BF),
                pltpu.VMEM((D, F), BF),
                pltpu.VMEM((F, D), BF),
                pltpu.VMEM(((S - PR) // 2, D), U32),
                pltpu.VMEM((A, D), F32),
                pltpu.VMEM((D, D), F32),
                pltpu.VMEM((D, 128), F32),
                pltpu.VMEM((8, D), F32),
                pltpu.VMEM((PR + CR, 256), F32),
                pltpu.VMEM((S, D), BF),
                pltpu.VMEM((7, PR // 4, KH), U32),
                pltpu.VMEM((7, 2, KH, 128), BF),
                pltpu.SMEM((1,), jnp.int32),
                pltpu.SemaphoreType.DMA((19,)),
                pltpu.SemaphoreType.DMA((1,)),
            ],
            compiler_params=pltpu.CompilerParams(vmem_limit_bytes=100 * 1024 * 1024,
                                                 disable_bounds_checks=True,
                                                 disable_semaphore_checks=True),
        )(x2, A_wqkv, A_wo, B_w_gate, B_w_up, B_w_down)
        return out.reshape(1, S, D)
    return fn


_impl = make()


@jax.jit
def pallas_recurrent_scan__linear_attn_block__geglu_ffn__prompt_kernel(
    A_x: jax.Array,
    A_wqkv: jax.Array,
    A_wo: jax.Array,
    B_x: jax.Array,
    B_w_gate: jax.Array,
    B_w_up: jax.Array,
    B_w_down: jax.Array,
):
    return _impl(A_x, A_wqkv, A_wo, B_x, B_w_gate, B_w_up, B_w_down)
```

```python
import jax
import jax.numpy as jnp
from jax import lax
import jax.experimental.pallas as pl
import jax.experimental.pallas.tpu as pltpu

S, D, F, H = 2048, 512, 1792, 32
DH = D // H
KH = D // 2
FH = F // 2
NJ = FH // 128
BF = jnp.bfloat16
F32 = jnp.float32
U32 = jnp.uint32
NT = (((1,), (1,)), ((), ()))


def _phi(t):
    return jnp.where(t > 0, t + 1.0, jnp.exp(t)) + 1e-6


def _gelu_mul(x, up):
    c0 = 0.7978845608028654
    c1 = 0.7978845608028654 * 0.044715
    t = jnp.tanh(x * (c0 + c1 * (x * x)))
    return (0.5 * x * up) * (1.0 + t)


def _rl(x, k):
    return pltpu.roll(x, k % 128, 1)


def _normalize(pq, zrow):
    n = pq.shape[0]
    lane = lax.broadcasted_iota(jnp.int32, (n, 128), 1)
    b0 = (lane & 1) != 0
    b1 = (lane & 2) != 0
    b2 = (lane & 4) != 0
    b3 = (lane & 8) != 0
    t = pq * zrow
    tb = [t[:, b * 128:(b + 1) * 128] for b in range(4)]
    m02 = jnp.where(b0, tb[0] + _rl(tb[0], 1), tb[2] + _rl(tb[2], -1))
    m13 = jnp.where(b0, tb[1] + _rl(tb[1], 1), tb[3] + _rl(tb[3], -1))
    u = jnp.where(b1, m02 + _rl(m02, 2), m13 + _rl(m13, -2))
    u = u + jnp.where(b2, _rl(u, 4), _rl(u, -4))
    u = u + jnp.where(b3, _rl(u, 8), _rl(u, -8))
    r = 1.0 / (u + 1e-6)
    r02 = jnp.where(b1, r, _rl(r, -2))
    r13 = jnp.where(b1, _rl(r, 2), r)
    rs = [jnp.where(b0, r02, _rl(r02, -1)), jnp.where(b0, r13, _rl(r13, -1)),
          jnp.where(b0, _rl(r02, 1), r02), jnp.where(b0, _rl(r13, 1), r13)]
    return jnp.concatenate([pq[:, b * 128:(b + 1) * 128] * rs[b] for b in range(4)], axis=1)


def _dot(a, b):
    return jnp.dot(a, b, preferred_element_type=F32)


def _sum8(x):
    n, c = x.shape
    return jnp.sum(x.reshape(n // 8, 8, c), axis=0)


def _acomb(a11, a12, a21, a22):
    return [(a11 + a22).astype(BF), (a21 + a22).astype(BF), a11.astype(BF), a22.astype(BF),
            (a11 + a12).astype(BF), (a21 - a11).astype(BF), (a12 - a22).astype(BF)]


def _bcomb(b11, b12, b21, b22):
    return [(b11 + b22).astype(BF), b11.astype(BF), (b12 - b22).astype(BF), (b21 - b11).astype(BF),
            b22.astype(BF), (b11 + b12).astype(BF), (b21 + b22).astype(BF)]


_A2B = (0, 2, 6, 5, 3, 4, 1)
_SC = ({0: 1, 3: 1, 4: -1, 6: 1}, {2: 1, 4: 1}, {1: 1, 3: 1}, {0: 1, 1: -1, 2: 1, 5: 1})


def make(A=896, E=128, NH=2, LAG=2, KSUB=256, P0=512, SA=(384, 128), WT=(2, 3, 4, 4), PB=128, QC=256,
         SEQ='c k0 q0 k1 q1 G01 k2 q2 k3 q3 p G23', LNF=2, QP1=(1, 7), QP2=(1, 7), QP3=(1, 7), NQ1=0,
         ORD=(4, 2, 1, 3, 0, 6, 5), QUAD=True):
    NL = 2
    assert NL * (sum(SA) + P0) == S
    PR = NL * P0
    CR = NL * SA[1]
    assert A + 128 + PR == S
    W = D // NH
    HB = PB // 2

    def scomb(m):
        out = []
        for q in _SC:
            acc, sign = None, 1
            for p in ORD:
                if p in q:
                    if acc is None:
                        acc, sign = m[p], q[p]
                    elif sign == 1:
                        acc = acc + m[p] if q[p] == 1 else acc - m[p]
                    else:
                        acc, sign = m[p] - acc, 1
            out.append(acc)
        return out

    def strassen(sa, tb):
        m = [None] * 7
        for p in ORD:
            m[p] = _dot(sa[p], tb[p])
        return scomb(m)

    def lcomb(v):
        nb = v.shape[0] // PB
        v1 = jnp.concatenate([v[b * PB:b * PB + HB] for b in range(nb)], axis=0)
        v2 = jnp.concatenate([v[b * PB + HB:(b + 1) * PB] for b in range(nb)], axis=0)
        return _acomb(v1[:, :KH], v1[:, KH:], v2[:, :KH], v2[:, KH:])

    def unhalves(c1, c2):
        nb = c1.shape[0] // HB
        return jnp.concatenate([t[b * HB:(b + 1) * HB] for b in range(nb) for t in (c1, c2)], axis=0)

    def rows2(c):
        return unhalves(c[0], c[2]), unhalves(c[1], c[3])

    def kernel(x_hbm, wqkv_hbm, wo_hbm, wg_hbm, wu_hbm, wd_hbm, o_hbm,
               x_v, wq_v, wk_v, wv_v, wo_v, wg_v, wu_v, wd_v, xn_v, kacc, g_acc, z_acc,
               zrow_v, pq_v, obuf, sa_v, cm_v, isem, osem):
        def xk_c(i):
            r0 = E if i >= 2 else 0
            return pltpu.make_async_copy(x_hbm.at[pl.ds(r0, A - r0), pl.ds(i * 128, 128)],
                                         x_v.at[pl.ds(r0, A - r0), pl.ds(i * 128, 128)], isem.at[i])

        def wk_c(i):
            return pltpu.make_async_copy(wqkv_hbm.at[pl.ds(i * 128, 128), pl.ds(D, D)],
                                         wk_v.at[pl.ds(i * 128, 128), :], isem.at[4 + i])

        def wq_c(b):
            return pltpu.make_async_copy(wqkv_hbm.at[:, pl.ds(b * 128, 128)], wq_v.at[:, pl.ds(b * 128, 128)],
                                         isem.at[8 + b])
        xe_c = pltpu.make_async_copy(x_hbm.at[pl.ds(0, E), pl.ds(256, 256)],
                                     x_v.at[pl.ds(0, E), pl.ds(256, 256)], isem.at[12])
        x2_c = pltpu.make_async_copy(x_hbm.at[pl.ds(A, S - A)], x_v.at[pl.ds(A, S - A)], isem.at[13])
        wv_c = pltpu.make_async_copy(wqkv_hbm.at[:, pl.ds(2 * D, D)], wv_v, isem.at[14])
        wo_c = pltpu.make_async_copy(wo_hbm, wo_v, isem.at[15])
        wg_c = pltpu.make_async_copy(wg_hbm, wg_v, isem.at[16])
        wu_c = pltpu.make_async_copy(wu_hbm, wu_v, isem.at[17])
        wd_c = pltpu.make_async_copy(wd_hbm, wd_v, isem.at[18])
        def ln(o, n):
            x = x_v[o:o + n, :].astype(F32)
            mu = jnp.sum(x, axis=-1, keepdims=True) * (1.0 / D)
            xc = x - mu
            var = jnp.sum(xc * xc, axis=-1, keepdims=True) * (1.0 / D)
            r = jnp.exp(-0.5 * jnp.log(var + 1e-5))
            xf = x * r - mu * r if (LNF == 2 and o >= A) else xc * r
            xn = xf.astype(BF)
            if o < S - PR:
                xn_v[o // 2:(o + n) // 2, :] = pltpu.bitcast(xn, U32)
            return xn, mu, r, xf

        def xn_ld(o, n):
            return pltpu.bitcast(xn_v[o // 2:(o + n) // 2, :], BF)

        def wops(cache, w_v, name, kh, nh, jt, r0=0, r1=None):
            r1 = kh if r1 is None else r1
            j = jt * 128
            r11 = w_v[r0:r1, j:j + 128]
            r22 = w_v[kh + r0:kh + r1, nh + j:nh + j + 128]
            key = (name, jt, r0)
            if key not in cache:
                b11 = r11.astype(F32)
                b12 = w_v[r0:r1, nh + j:nh + j + 128].astype(F32)
                b21 = w_v[kh + r0:kh + r1, j:j + 128].astype(F32)
                b22 = r22.astype(F32)
                cache[key] = [t.astype(BF) for t in (b11 + b22, b12 - b22, b21 - b11, b11 + b12, b21 + b22)]
            c = cache[key]
            return [c[0], r11, c[1], c[2], r22, c[3], c[4]]

        class Tile:
            def __init__(self, cache, h0, n, pq_off=None, hq=None):
                self.cache, self.h0, self.n, self.pq_off = cache, h0, n, pq_off
                if hq is not None:
                    hr = pl.ds(pl.multiple_of(hq, 8), n // 4)
                    self.sa = [pltpu.bitcast(sa_v[p, hr, :], BF) for p in range(7)]
                else:
                    xn = pltpu.bitcast(xn_v[pl.ds(pl.multiple_of(h0, 8), n // 2), :], BF)
                    self.sa = lcomb(xn.astype(F32))
                self.aparts = []
                self.gs = []

            def qjobs(self):
                return [(self, b, min(QC, self.n - b)) for b in range(0, self.n, QC)]

            def qchunk(self, b, m):
                sc = self.sa if m == self.n else [t[b // 2:(b + m) // 2] for t in self.sa]
                if self.pq_off is not None:
                    rw = pl.ds(pl.multiple_of(2 * self.h0 + b + self.pq_off, 16), m)
                    p0, p2 = pq_v[rw, 0:128], pq_v[rw, 128:256]
                else:
                    p0, p2 = [_phi(t) for t in rows2(strassen(sc, wops(self.cache, wq_v, 'q', KH, KH, 0)))]
                p1, p3 = [_phi(t) for t in rows2(strassen(sc, wops(self.cache, wq_v, 'q', KH, KH, 1)))]
                self.aparts.append(_normalize(jnp.concatenate([p0, p1, p2, p3], axis=1), zrow_v[0:1, :]))

            def ffn(self, jobs, qp, qe):
                cache, sa = self.cache, self.sa
                done = [0]

                def qupto(pos):
                    if pos >= qp:
                        want = min(len(jobs), -(-(pos - qp + 1) * len(jobs) // (qe + 1 - qp)))
                        while done[0] < want:
                            t, b, m = jobs[done[0]]
                            t.qchunk(b, m)
                            done[0] += 1

                hs = []
                for jt in range(NJ):
                    qupto(jt)
                    gq = strassen(sa, wops(cache, wg_v, 'g', KH, FH, jt))
                    uq = strassen(sa, wops(cache, wu_v, 'u', KH, FH, jt))
                    hs.append(_acomb(*[_gelu_mul(gq[t], uq[t]) for t in range(4)]))
                for jt in range(2):
                    wd = [wops(cache, wd_v, 'd', FH, KH, jt, k * 128, (k + 1) * 128) for k in range(NJ)]
                    m = [None] * 7
                    for pi, p in enumerate(ORD):
                        qupto(NJ + jt * 7 + pi)
                        for k in range(NJ):
                            t = _dot(hs[k][p], wd[k][p])
                            m[p] = t if m[p] is None else m[p] + t
                    for y in rows2(scomb(m)):
                        hy = 0.5 * y
                        self.gs.append(hy * (1.0 + jnp.tanh(hy)))

            def out(self, split_out):
                row = pl.ds(pl.multiple_of(2 * self.h0, 16), self.n)
                aa = lcomb(jnp.concatenate(self.aparts, axis=0))
                if split_out and QUAD:
                    assert self.n == PB
                    for jt in range(2):
                        sq = strassen(aa, [cm_v[p, jt] for p in range(7)])
                        for q in (1, 2, 0, 3):
                            c0 = (q % 2) * KH + jt * 128
                            r0 = (q // 2) * HB
                            rq = pl.ds(pl.multiple_of(2 * self.h0 + r0, 16), HB)
                            obuf[rq, c0:c0 + 128] = (x_v[rq, c0:c0 + 128].astype(F32) + sq[q]
                                                     * self.gs[2 * jt + q % 2][r0:r0 + HB]).astype(BF)
                            pltpu.make_async_copy(obuf.at[rq, pl.ds(c0, 128)], o_hbm.at[rq, pl.ds(c0, 128)],
                                                  osem.at[0]).start()
                    return
                for jt in range(2):
                    ss = rows2(strassen(aa, [cm_v[p, jt] for p in range(7)]))
                    for t in range(2):
                        c0 = t * KH + jt * 128
                        obuf[row, c0:c0 + 128] = (x_v[row, c0:c0 + 128].astype(F32)
                                                  + ss[t] * self.gs[2 * jt + t]).astype(BF)
                        if split_out:
                            pltpu.make_async_copy(obuf.at[row, pl.ds(c0, 128)], o_hbm.at[row, pl.ds(c0, 128)],
                                                  osem.at[0]).start()
                if not split_out:
                    pltpu.make_async_copy(obuf.at[row], o_hbm.at[row], osem.at[0]).start()

        def body(i):
            cache = {}
            t1 = Tile(cache, (S - PR) // 2 + i * (P0 // 2), P0, PR - S, i * (P0 // 4))
            j1 = t1.qjobs()
            t1.ffn(j1[:NQ1], *QP1)
            if NQ1 >= len(j1):
                t1.out(False)
            t2 = Tile(cache, CR // 2 + i * (SA[0] // 2), SA[0])
            t2.ffn(j1[NQ1:] + t2.qjobs(), *QP2)
            if NQ1 < len(j1):
                t1.out(False)
            t2.out(False)
            t3 = Tile(cache, i * (SA[1] // 2), SA[1], PR)
            t3.ffn(t3.qjobs(), *QP3)
            t3.out(True)

        def prologue():
            for i in range(4):
                wk_c(i).start()
                xk_c(i).start()
                if i == 1:
                    xe_c.start()
            for c in (x2_c, wq_c(0), wq_c(2), wv_c, wo_c, wq_c(1), wq_c(3), wg_c, wu_c, wd_c):
                c.start()

            wkts = [None] * 4

            def wkt(blk):
                for i in range(4):
                    if WT[i] == blk:
                        wkts[i] = wk_v[i * 128:(i + 1) * 128, :].astype(F32).T

            wk_c(0).wait()
            xk_c(0).wait()
            kacc[...] = _dot(x_v[0:A, 0:128], wk_v[0:128, :])
            wkt(2)
            cs8 = _sum8(wk_v[0:128, :].astype(F32))

            wk_c(1).wait()
            xk_c(1).wait()
            xe_c.wait()
            lns = {j: ln(j * 128, 128) for j in range(E // 128)}
            kacc[...] += _dot(x_v[0:A, 128:256], wk_v[128:256, :])
            wkt(3)
            cs8 = cs8 + _sum8(wk_v[128:256, :].astype(F32))

            for i in (2, 3):
                wk_c(i).wait()
                xk_c(i).wait()
            cs = jnp.sum(cs8 + _sum8(wk_v[256:512, :].astype(F32)), axis=0, keepdims=True)
            wkt(4)
            zn = [None] * NH
            pks = {}
            units = [(j, h) for j in range(A // 128) for h in range(NH)]

            def kunit(j, h):
                o = j * 128
                cl = slice(h * W, (h + 1) * W)
                kraw = kacc[o:o + 128, cl] + _dot(x_v[o:o + 128, 256:512], wk_v[256:512, cl])
                if j not in lns:
                    lns[j] = ln(o, 128)
                _, mu, r, _ = lns[j]
                pk = _phi((kraw - mu * cs[:, cl]) * r)
                zp = _sum8(pk)
                zn[h] = zp if zn[h] is None else zn[h] + zp
                pks[(j, h)] = pk.T.astype(BF)

            def gunit(j, h):
                gp = _dot(pks[(j, h)], lns[j][0] if j * 128 >= E else xn_ld(j * 128, 128))
                if j == 0:
                    g_acc[h * W:(h + 1) * W, :] = gp
                else:
                    g_acc[h * W:(h + 1) * W, :] += gp

            for t in range(len(units) + LAG):
                if t < len(units):
                    kunit(*units[t])
                if t >= LAG:
                    gunit(*units[t - LAG])
            znat = jnp.concatenate(zn, axis=1)

            x2_c.wait()
            wq_c(0).wait()
            wq_c(2).wait()
            wv_c.wait()
            wo_c.wait()
            wkt(5)
            wf = jnp.concatenate(wkts, axis=1)
            wkc = _bcomb(wf[:KH, :KH], wf[KH:, :KH], wf[:KH, KH:], wf[KH:, KH:])
            wq0 = wops({}, wq_v, 'q', KH, KH, 0)
            kd = {}
            zfirst = True
            for step in SEQ.split():
                if step == 'c':
                    xe = xn_ld(0, CR)
                    pq_v[PR:PR + CR, 0:128] = _phi(_dot(xe, wq_v[:, 0:128]))
                    pq_v[PR:PR + CR, 128:256] = _phi(_dot(xe, wq_v[:, 256:384]))
                elif step == 'p':
                    xn_l = ln(A, 128)[0]
                    t = _phi(lax.dot_general(wf.astype(BF), xn_l, NT, preferred_element_type=F32))
                    if zfirst:
                        z_acc[...] = t
                    else:
                        z_acc[...] += t
                    zfirst = False
                    pk_l = [t[b * 128:(b + 1) * 128, :].astype(BF) for b in range(4)]
                elif step[0] == 'q':
                    ci = int(step[1:])
                    lo, hi = rows2([_phi(t) for t in strassen(kd[ci][1], wq0)])
                    pq_v[ci * KSUB:(ci + 1) * KSUB, 0:128] = lo
                    pq_v[ci * KSUB:(ci + 1) * KSUB, 128:256] = hi
                elif step[0] == 'k':
                    ci = int(step[1:])
                    h = KSUB // 2
                    sa = lcomb(ln(S - PR + ci * KSUB, KSUB)[3])
                    for p in range(7):
                        sa_v[p, ci * h // 2:(ci + 1) * h // 2, :] = pltpu.bitcast(sa[p], U32)
                    m = [None] * 7
                    for p in ORD:
                        m[p] = lax.dot_general(wkc[p], sa[p], NT, preferred_element_type=F32)
                    c = [_phi(t) for t in scomb(m)]
                    for (r0, t) in ((0, c[0] + c[2]), (KH, c[1] + c[3])):
                        zp = t[:, 0:128]
                        for cc in range(1, h // 128):
                            zp = zp + t[:, cc * 128:(cc + 1) * 128]
                        if zfirst:
                            z_acc[r0:r0 + KH, :] = zp
                        else:
                            z_acc[r0:r0 + KH, :] += zp
                    zfirst = False
                    kd[ci] = (_acomb(c[0], c[2], c[1], c[3]), sa)
                else:
                    m = [None] * 7
                    for p in ORD:
                        for ch in step[1:]:
                            pa, sa = kd[int(ch)]
                            t = _dot(pa[p], sa[_A2B[p]])
                            m[p] = t if m[p] is None else m[p] + t
                    c = scomb(m)
                    g_acc[0:KH, 0:KH] += c[0]
                    g_acc[0:KH, KH:D] += c[1]
                    g_acc[KH:D, 0:KH] += c[2]
                    g_acc[KH:D, KH:D] += c[3]
            zrow = jnp.sum(_sum8(z_acc[...].T) + znat, axis=0, keepdims=True)
            zrow_v[...] = jnp.broadcast_to(zrow, (8, D))

            rr = lax.broadcasted_iota(jnp.int32, (128, 128), 0) // DH
            cc = lax.broadcasted_iota(jnp.int32, (128, 128), 1) // DH
            mask = rr == cc
            mb = [None] * 4

            def gblk(b):
                return g_acc[b * 128:(b + 1) * 128, :] + _dot(pk_l[b], xn_l)

            def kvblk(gb, b):
                kvb = _dot(gb.astype(BF), wv_v[:, b * 128:(b + 1) * 128])
                return jnp.where(mask, kvb, 0.0).astype(BF)

            def mblk(kvb, b):
                mb[b] = _dot(kvb, wo_v[b * 128:(b + 1) * 128, :])
                if b >= 2:
                    top, bot = mb[b - 2], mb[b]
                    for jt in range(2):
                        j = jt * 128
                        c = _bcomb(top[:, j:j + 128], top[:, KH + j:KH + j + 128],
                                   bot[:, j:j + 128], bot[:, KH + j:KH + j + 128])
                        for p in range(7):
                            cm_v[p, jt, (b - 2) * 128:(b - 1) * 128, :] = c[p]

            g0 = gblk(0)
            g1 = gblk(1)
            kv0 = kvblk(g0, 0)
            g2 = gblk(2)
            kv1 = kvblk(g1, 1)
            g3 = gblk(3)
            kv2 = kvblk(g2, 2)
            mblk(kv0, 0)
            kv3 = kvblk(g3, 3)
            mblk(kv1, 1)
            mblk(kv2, 2)
            mblk(kv3, 3)

            wq_c(1).wait()
            wq_c(3).wait()
            wg_c.wait()
            wu_c.wait()
            wd_c.wait()

        step = pl.program_id(0)
        pl.when(step == 0)(prologue)
        body(step)

        @pl.when(step == NL - 1)
        def _():
            pltpu.make_async_copy(obuf, o_hbm, osem.at[0]).wait()

    def fn(A_x, A_wqkv, A_wo, B_x, B_w_gate, B_w_up, B_w_down):
        x2 = A_x.reshape(S, D)
        out = pl.pallas_call(
            kernel,
            out_shape=jax.ShapeDtypeStruct((S, D), BF),
            grid=(NL,),
            in_specs=[pl.BlockSpec(memory_space=pl.ANY)] * 6,
            out_specs=pl.BlockSpec(memory_space=pl.ANY),
            scratch_shapes=[
                pltpu.VMEM((S, D), BF),
                pltpu.VMEM((D, D), BF),
                pltpu.VMEM((D, D), BF),
                pltpu.VMEM((D, D), BF),
                pltpu.VMEM((D, D), BF),
                pltpu.VMEM((D, F), BF),
                pltpu.VMEM((D, F), BF),
                pltpu.VMEM((F, D), BF),
                pltpu.VMEM(((S - PR) // 2, D), U32),
                pltpu.VMEM((A, D), F32),
                pltpu.VMEM((D, D), F32),
                pltpu.VMEM((D, 128), F32),
                pltpu.VMEM((8, D), F32),
                pltpu.VMEM((PR + CR, 256), F32),
                pltpu.VMEM((S, D), BF),
                pltpu.VMEM((7, PR // 4, KH), U32),
                pltpu.VMEM((7, 2, KH, 128), BF),
                pltpu.SemaphoreType.DMA((19,)),
                pltpu.SemaphoreType.DMA((1,)),
            ],
            compiler_params=pltpu.CompilerParams(dimension_semantics=("arbitrary",),
                                                 vmem_limit_bytes=100 * 1024 * 1024,
                                                 disable_bounds_checks=True,
                                                 disable_semaphore_checks=True),
        )(x2, A_wqkv, A_wo, B_w_gate, B_w_up, B_w_down)
        return out.reshape(1, S, D)
    return fn


_impl = make()


@jax.jit
def pallas_recurrent_scan__linear_attn_block__geglu_ffn__prompt_kernel(
    A_x: jax.Array,
    A_wqkv: jax.Array,
    A_wo: jax.Array,
    B_x: jax.Array,
    B_w_gate: jax.Array,
    B_w_up: jax.Array,
    B_w_down: jax.Array,
):
    return _impl(A_x, A_wqkv, A_wo, B_x, B_w_gate, B_w_up, B_w_down)
```

```python
import jax
import jax.numpy as jnp
from jax import lax
import jax.experimental.pallas as pl
import jax.experimental.pallas.tpu as pltpu

S, D, F, H = 2048, 512, 1792, 32
DH = D // H
KH = D // 2
FH = F // 2
NJ = FH // 128
BF = jnp.bfloat16
F32 = jnp.float32
U32 = jnp.uint32
NT = (((1,), (1,)), ((), ()))

NL = 2
A = 896
E = 128
W = 256
LAG = 2
KSUB = 256
T1, T2, T3 = 512, 384, 128
PR = NL * T1
CR = NL * T3
PB = 128
HB = PB // 2
QC = 256
SEQ = ('c', 'k0', 'q0', 'k1', 'q1', 'G01', 'k2', 'q2', 'k3', 'q3', 'G23', 'p')
ORD = (4, 2, 1, 3, 0, 6, 5)
assert NL * (T1 + T2 + T3) == S and A + 128 + PR == S and T3 == PB


def _phi(t):
    return jnp.where(t > 0, t + 1.0, jnp.exp(t)) + 1e-6


def _gelu_mul(x, up):
    c0 = 0.7978845608028654
    c1 = 0.7978845608028654 * 0.044715
    t = jnp.tanh(x * (c0 + c1 * (x * x)))
    return (0.5 * x * up) * (1.0 + t)


def _rl(x, k):
    return pltpu.roll(x, k % 128, 1)


def _normalize(pq, zrow):
    n = pq.shape[0]
    lane = lax.broadcasted_iota(jnp.int32, (n, 128), 1)
    b0 = (lane & 1) != 0
    b1 = (lane & 2) != 0
    b2 = (lane & 4) != 0
    b3 = (lane & 8) != 0
    t = pq * zrow
    tb = [t[:, b * 128:(b + 1) * 128] for b in range(4)]
    m02 = jnp.where(b0, tb[0] + _rl(tb[0], 1), tb[2] + _rl(tb[2], -1))
    m13 = jnp.where(b0, tb[1] + _rl(tb[1], 1), tb[3] + _rl(tb[3], -1))
    u = jnp.where(b1, m02 + _rl(m02, 2), m13 + _rl(m13, -2))
    u = u + jnp.where(b2, _rl(u, 4), _rl(u, -4))
    u = u + jnp.where(b3, _rl(u, 8), _rl(u, -8))
    r = 1.0 / (u + 1e-6)
    r02 = jnp.where(b1, r, _rl(r, -2))
    r13 = jnp.where(b1, _rl(r, 2), r)
    rs = [jnp.where(b0, r02, _rl(r02, -1)), jnp.where(b0, r13, _rl(r13, -1)),
          jnp.where(b0, _rl(r02, 1), r02), jnp.where(b0, _rl(r13, 1), r13)]
    return jnp.concatenate([pq[:, b * 128:(b + 1) * 128] * rs[b] for b in range(4)], axis=1)


def _dot(a, b):
    return jnp.dot(a, b, preferred_element_type=F32)


def _sum8(x):
    n, c = x.shape
    return jnp.sum(x.reshape(n // 8, 8, c), axis=0)


def _acomb(a11, a12, a21, a22):
    return [(a11 + a22).astype(BF), (a21 + a22).astype(BF), a11.astype(BF), a22.astype(BF),
            (a11 + a12).astype(BF), (a21 - a11).astype(BF), (a12 - a22).astype(BF)]


def _bcomb(b11, b12, b21, b22):
    return [(b11 + b22).astype(BF), b11.astype(BF), (b12 - b22).astype(BF), (b21 - b11).astype(BF),
            b22.astype(BF), (b11 + b12).astype(BF), (b21 + b22).astype(BF)]


_A2B = (0, 2, 6, 5, 3, 4, 1)
_SC = ({0: 1, 3: 1, 4: -1, 6: 1}, {2: 1, 4: 1}, {1: 1, 3: 1}, {0: 1, 1: -1, 2: 1, 5: 1})


def _scomb(m):
    out = []
    for q in _SC:
        acc, sign = None, 1
        for p in ORD:
            if p in q:
                if acc is None:
                    acc, sign = m[p], q[p]
                elif sign == 1:
                    acc = acc + m[p] if q[p] == 1 else acc - m[p]
                else:
                    acc, sign = m[p] - acc, 1
        out.append(acc)
    return out


def _strassen(sa, tb):
    m = [None] * 7
    for p in ORD:
        m[p] = _dot(sa[p], tb[p])
    return _scomb(m)


def _lcomb(v):
    nb = v.shape[0] // PB
    v1 = jnp.concatenate([v[b * PB:b * PB + HB] for b in range(nb)], axis=0)
    v2 = jnp.concatenate([v[b * PB + HB:(b + 1) * PB] for b in range(nb)], axis=0)
    return _acomb(v1[:, :KH], v1[:, KH:], v2[:, :KH], v2[:, KH:])


def _unhalves(c1, c2):
    nb = c1.shape[0] // HB
    return jnp.concatenate([t[b * HB:(b + 1) * HB] for b in range(nb) for t in (c1, c2)], axis=0)


def _rows2(c):
    return _unhalves(c[0], c[2]), _unhalves(c[1], c[3])


def _wops(cache, w_v, name, kh, nh, jt, r0=0, r1=None):
    r1 = kh if r1 is None else r1
    j = jt * 128
    r11 = w_v[r0:r1, j:j + 128]
    r22 = w_v[kh + r0:kh + r1, nh + j:nh + j + 128]
    key = (name, jt, r0)
    if key not in cache:
        b11 = r11.astype(F32)
        b12 = w_v[r0:r1, nh + j:nh + j + 128].astype(F32)
        b21 = w_v[kh + r0:kh + r1, j:j + 128].astype(F32)
        b22 = r22.astype(F32)
        cache[key] = [t.astype(BF) for t in (b11 + b22, b12 - b22, b21 - b11, b11 + b12, b21 + b22)]
    c = cache[key]
    return [c[0], r11, c[1], c[2], r22, c[3], c[4]]


def _kernel(x_hbm, wqkv_hbm, wo_hbm, wg_hbm, wu_hbm, wd_hbm, o_hbm,
            x_v, wq_v, wk_v, wv_v, wo_v, wg_v, wu_v, wd_v, xn_v, kacc, g_acc, z_acc,
            zrow_v, pq_v, obuf, sa_v, cm_v, isem, osem):

    def ln(o, n):
        x = x_v[o:o + n, :].astype(F32)
        mu = jnp.sum(x, axis=-1, keepdims=True) * (1.0 / D)
        xc = x - mu
        var = jnp.sum(xc * xc, axis=-1, keepdims=True) * (1.0 / D)
        r = jnp.exp(-0.5 * jnp.log(var + 1e-5))
        xf = xc * r
        xn = xf.astype(BF)
        if o < S - PR:
            xn_v[o // 2:(o + n) // 2, :] = pltpu.bitcast(xn, U32)
        return xn, mu, r, xf

    def xn_ld(o, n):
        return pltpu.bitcast(xn_v[o // 2:(o + n) // 2, :], BF)

    def prologue():
        def xk_c(i):
            r0 = E if i >= 2 else 0
            return pltpu.make_async_copy(x_hbm.at[pl.ds(r0, A - r0), pl.ds(i * 128, 128)],
                                         x_v.at[pl.ds(r0, A - r0), pl.ds(i * 128, 128)], isem.at[i])

        def wk_c(i):
            return pltpu.make_async_copy(wqkv_hbm.at[pl.ds(i * 128, 128), pl.ds(D, D)],
                                         wk_v.at[pl.ds(i * 128, 128), :], isem.at[4 + i])

        def wq_c(b):
            return pltpu.make_async_copy(wqkv_hbm.at[:, pl.ds(b * 128, 128)],
                                         wq_v.at[:, pl.ds(b * 128, 128)], isem.at[8 + b])
        xe_c = pltpu.make_async_copy(x_hbm.at[pl.ds(0, E), pl.ds(256, 256)],
                                     x_v.at[pl.ds(0, E), pl.ds(256, 256)], isem.at[12])
        x2_c = pltpu.make_async_copy(x_hbm.at[pl.ds(A, S - A)], x_v.at[pl.ds(A, S - A)], isem.at[13])
        wv_c = pltpu.make_async_copy(wqkv_hbm.at[:, pl.ds(2 * D, D)], wv_v, isem.at[14])
        wo_c = pltpu.make_async_copy(wo_hbm, wo_v, isem.at[15])
        wg_c = pltpu.make_async_copy(wg_hbm, wg_v, isem.at[16])
        wu_c = pltpu.make_async_copy(wu_hbm, wu_v, isem.at[17])
        wd_c = pltpu.make_async_copy(wd_hbm, wd_v, isem.at[18])
        for i in range(4):
            wk_c(i).start()
            xk_c(i).start()
            if i == 1:
                xe_c.start()
        for c in (x2_c, wq_c(0), wq_c(2), wv_c, wo_c, wq_c(1), wq_c(3), wg_c, wu_c, wd_c):
            c.start()

        def wkt(i):
            return wk_v[i * 128:(i + 1) * 128, :].astype(F32).T

        wk_c(0).wait()
        xk_c(0).wait()
        kacc[...] = _dot(x_v[0:A, 0:128], wk_v[0:128, :])
        wkts = [wkt(0)]
        cs8 = _sum8(wk_v[0:128, :].astype(F32))

        wk_c(1).wait()
        xk_c(1).wait()
        xe_c.wait()
        lns = {j: ln(j * 128, 128) for j in range(E // 128)}
        kacc[...] += _dot(x_v[0:A, 128:256], wk_v[128:256, :])
        wkts.append(wkt(1))
        cs8 = cs8 + _sum8(wk_v[128:256, :].astype(F32))

        for i in (2, 3):
            wk_c(i).wait()
            xk_c(i).wait()
        cs = jnp.sum(cs8 + _sum8(wk_v[256:512, :].astype(F32)), axis=0, keepdims=True)
        wkts += [wkt(2), wkt(3)]
        zn = [None] * (D // W)
        pks = {}
        units = [(j, h) for j in range(A // 128) for h in range(D // W)]

        def kunit(j, h):
            o = j * 128
            cl = slice(h * W, (h + 1) * W)
            kraw = kacc[o:o + 128, cl] + _dot(x_v[o:o + 128, 256:512], wk_v[256:512, cl])
            if j not in lns:
                lns[j] = ln(o, 128)
            _, mu, r, _ = lns[j]
            pk = _phi((kraw - mu * cs[:, cl]) * r)
            zp = _sum8(pk)
            zn[h] = zp if zn[h] is None else zn[h] + zp
            pks[(j, h)] = pk.T.astype(BF)

        def gunit(j, h):
            gp = _dot(pks[(j, h)], lns[j][0] if j * 128 >= E else xn_ld(j * 128, 128))
            if j == 0:
                g_acc[h * W:(h + 1) * W, :] = gp
            else:
                g_acc[h * W:(h + 1) * W, :] += gp

        for t in range(len(units) + LAG):
            if t < len(units):
                kunit(*units[t])
            if t >= LAG:
                gunit(*units[t - LAG])
        znat = jnp.concatenate(zn, axis=1)

        x2_c.wait()
        wq_c(0).wait()
        wq_c(2).wait()
        wv_c.wait()
        wo_c.wait()
        wf = jnp.concatenate(wkts, axis=1)
        wkc = _bcomb(wf[:KH, :KH], wf[KH:, :KH], wf[:KH, KH:], wf[KH:, KH:])
        wq0 = _wops({}, wq_v, 'q', KH, KH, 0)
        kd = {}
        hk = KSUB // 2
        for op in SEQ:
            if op == 'c':
                xe = xn_ld(0, CR)
                pq_v[PR:PR + CR, 0:128] = _phi(_dot(xe, wq_v[:, 0:128]))
                pq_v[PR:PR + CR, 128:256] = _phi(_dot(xe, wq_v[:, 256:384]))
            elif op == 'p':
                xn_l = ln(A, 128)[0]
                t = _phi(lax.dot_general(wf.astype(BF), xn_l, NT, preferred_element_type=F32))
                z_acc[...] += t
                pk_l = [t[b * 128:(b + 1) * 128, :].astype(BF) for b in range(4)]
            elif op[0] == 'q':
                ci = int(op[1:])
                lo, hi = _rows2([_phi(t) for t in _strassen(kd[ci][1], wq0)])
                pq_v[ci * KSUB:(ci + 1) * KSUB, 0:128] = lo
                pq_v[ci * KSUB:(ci + 1) * KSUB, 128:256] = hi
            elif op[0] == 'k':
                ci = int(op[1:])
                sa = _lcomb(ln(S - PR + ci * KSUB, KSUB)[3])
                for p in range(7):
                    sa_v[p, ci * hk // 2:(ci + 1) * hk // 2, :] = pltpu.bitcast(sa[p], U32)
                m = [None] * 7
                for p in ORD:
                    m[p] = lax.dot_general(wkc[p], sa[p], NT, preferred_element_type=F32)
                c = [_phi(t) for t in _scomb(m)]
                for (r0, zp) in ((0, c[0] + c[2]), (KH, c[1] + c[3])):
                    if ci == 0:
                        z_acc[r0:r0 + KH, :] = zp
                    else:
                        z_acc[r0:r0 + KH, :] += zp
                kd[ci] = (_acomb(c[0], c[2], c[1], c[3]), sa)
            else:
                m = [None] * 7
                for p in ORD:
                    for ch in op[1:]:
                        pa, sa = kd[int(ch)]
                        t = _dot(pa[p], sa[_A2B[p]])
                        m[p] = t if m[p] is None else m[p] + t
                c = _scomb(m)
                g_acc[0:KH, 0:KH] += c[0]
                g_acc[0:KH, KH:D] += c[1]
                g_acc[KH:D, 0:KH] += c[2]
                g_acc[KH:D, KH:D] += c[3]
        zrow = jnp.sum(_sum8(z_acc[...].T) + znat, axis=0, keepdims=True)
        zrow_v[...] = jnp.broadcast_to(zrow, (8, D))

        rr = lax.broadcasted_iota(jnp.int32, (128, 128), 0) // DH
        cc = lax.broadcasted_iota(jnp.int32, (128, 128), 1) // DH
        mask = rr == cc
        mb = [None] * 4

        def gblk(b):
            return g_acc[b * 128:(b + 1) * 128, :] + _dot(pk_l[b], xn_l)

        def kvblk(gb, b):
            kvb = _dot(gb.astype(BF), wv_v[:, b * 128:(b + 1) * 128])
            return jnp.where(mask, kvb, 0.0).astype(BF)

        def mblk(kvb, b):
            mb[b] = _dot(kvb, wo_v[b * 128:(b + 1) * 128, :])
            if b >= 2:
                top, bot = mb[b - 2], mb[b]
                for jt in range(2):
                    j = jt * 128
                    c = _bcomb(top[:, j:j + 128], top[:, KH + j:KH + j + 128],
                               bot[:, j:j + 128], bot[:, KH + j:KH + j + 128])
                    for p in range(7):
                        cm_v[p, jt, (b - 2) * 128:(b - 1) * 128, :] = c[p]

        g0 = gblk(0)
        g1 = gblk(1)
        kv0 = kvblk(g0, 0)
        g2 = gblk(2)
        kv1 = kvblk(g1, 1)
        g3 = gblk(3)
        kv2 = kvblk(g2, 2)
        mblk(kv0, 0)
        kv3 = kvblk(g3, 3)
        mblk(kv1, 1)
        mblk(kv2, 2)
        mblk(kv3, 3)

        wq_c(1).wait()
        wq_c(3).wait()
        wg_c.wait()
        wu_c.wait()
        wd_c.wait()

    cache = {}

    class Tile:
        def __init__(self, h0, n, pq_off=None, hq=None):
            self.h0, self.n, self.pq_off = h0, n, pq_off
            if hq is not None:
                hr = pl.ds(pl.multiple_of(hq, 8), n // 4)
                self.sa = [pltpu.bitcast(sa_v[p, hr, :], BF) for p in range(7)]
            else:
                xn = pltpu.bitcast(xn_v[pl.ds(pl.multiple_of(h0, 8), n // 2), :], BF)
                self.sa = _lcomb(xn.astype(F32))
            self.aparts = []
            self.gs = []

        def qjobs(self):
            return [(self, b, min(QC, self.n - b)) for b in range(0, self.n, QC)]

        def qchunk(self, b, m):
            sc = self.sa if m == self.n else [t[b // 2:(b + m) // 2] for t in self.sa]
            if self.pq_off is not None:
                rw = pl.ds(pl.multiple_of(2 * self.h0 + b + self.pq_off, 16), m)
                p0, p2 = pq_v[rw, 0:128], pq_v[rw, 128:256]
            else:
                p0, p2 = [_phi(t) for t in _rows2(_strassen(sc, _wops(cache, wq_v, 'q', KH, KH, 0)))]
            p1, p3 = [_phi(t) for t in _rows2(_strassen(sc, _wops(cache, wq_v, 'q', KH, KH, 1)))]
            self.aparts.append(_normalize(jnp.concatenate([p0, p1, p2, p3], axis=1), zrow_v[0:1, :]))

        def ffn(self, jobs):
            done = 0
            hs = []
            for jt in range(NJ + 1):
                while done < -(-jt * len(jobs) // NJ):
                    t, b, m = jobs[done]
                    t.qchunk(b, m)
                    done += 1
                if jt < NJ:
                    gq = _strassen(self.sa, _wops(cache, wg_v, 'g', KH, FH, jt))
                    uq = _strassen(self.sa, _wops(cache, wu_v, 'u', KH, FH, jt))
                    hs.append(_acomb(*[_gelu_mul(gq[t], uq[t]) for t in range(4)]))
            for jt in range(2):
                wd = [_wops(cache, wd_v, 'd', FH, KH, jt, k * 128, (k + 1) * 128) for k in range(NJ)]
                m = [None] * 7
                for p in ORD:
                    for k in range(NJ):
                        t = _dot(hs[k][p], wd[k][p])
                        m[p] = t if m[p] is None else m[p] + t
                for y in _rows2(_scomb(m)):
                    hy = 0.5 * y
                    self.gs.append(hy * (1.0 + jnp.tanh(hy)))

        def out(self, fine):
            aa = _lcomb(jnp.concatenate(self.aparts, axis=0))
            row = pl.ds(pl.multiple_of(2 * self.h0, 16), self.n)
            for jt in range(2):
                sq = _strassen(aa, [cm_v[p, jt] for p in range(7)])
                if fine:
                    for q in (1, 2, 0, 3):
                        c0 = (q % 2) * KH + jt * 128
                        r0 = (q // 2) * HB
                        rq = pl.ds(pl.multiple_of(2 * self.h0 + r0, 16), HB)
                        obuf[rq, c0:c0 + 128] = (x_v[rq, c0:c0 + 128].astype(F32)
                                                 + sq[q] * self.gs[2 * jt + q % 2][r0:r0 + HB]).astype(BF)
                        pltpu.make_async_copy(obuf.at[rq, pl.ds(c0, 128)], o_hbm.at[rq, pl.ds(c0, 128)],
                                              osem.at[0]).start()
                else:
                    ss = _rows2(sq)
                    for t in range(2):
                        c0 = t * KH + jt * 128
                        obuf[row, c0:c0 + 128] = (x_v[row, c0:c0 + 128].astype(F32)
                                                  + ss[t] * self.gs[2 * jt + t]).astype(BF)
            if not fine:
                pltpu.make_async_copy(obuf.at[row], o_hbm.at[row], osem.at[0]).start()

    i = pl.program_id(0)
    pl.when(i == 0)(prologue)

    t1 = Tile((S - PR) // 2 + i * (T1 // 2), T1, PR - S, i * (T1 // 4))
    t1.ffn([])
    t2 = Tile(CR // 2 + i * (T2 // 2), T2)
    t2.ffn(t1.qjobs() + t2.qjobs())
    t1.out(False)
    t2.out(False)
    t3 = Tile(i * (T3 // 2), T3, PR)
    t3.ffn(t3.qjobs())
    t3.out(True)

    @pl.when(i == NL - 1)
    def _():
        pltpu.make_async_copy(obuf, o_hbm, osem.at[0]).wait()


@jax.jit
def pallas_recurrent_scan__linear_attn_block__geglu_ffn__prompt_kernel(
    A_x: jax.Array,
    A_wqkv: jax.Array,
    A_wo: jax.Array,
    B_x: jax.Array,
    B_w_gate: jax.Array,
    B_w_up: jax.Array,
    B_w_down: jax.Array,
):
    out = pl.pallas_call(
        _kernel,
        out_shape=jax.ShapeDtypeStruct((S, D), BF),
        grid=(NL,),
        in_specs=[pl.BlockSpec(memory_space=pl.ANY)] * 6,
        out_specs=pl.BlockSpec(memory_space=pl.ANY),
        scratch_shapes=[
            pltpu.VMEM((S, D), BF),
            pltpu.VMEM((D, D), BF),
            pltpu.VMEM((D, D), BF),
            pltpu.VMEM((D, D), BF),
            pltpu.VMEM((D, D), BF),
            pltpu.VMEM((D, F), BF),
            pltpu.VMEM((D, F), BF),
            pltpu.VMEM((F, D), BF),
            pltpu.VMEM(((S - PR) // 2, D), U32),
            pltpu.VMEM((A, D), F32),
            pltpu.VMEM((D, D), F32),
            pltpu.VMEM((D, 128), F32),
            pltpu.VMEM((8, D), F32),
            pltpu.VMEM((PR + CR, 256), F32),
            pltpu.VMEM((S, D), BF),
            pltpu.VMEM((7, PR // 4, KH), U32),
            pltpu.VMEM((7, 2, KH, 128), BF),
            pltpu.SemaphoreType.DMA((19,)),
            pltpu.SemaphoreType.DMA((1,)),
        ],
        compiler_params=pltpu.CompilerParams(dimension_semantics=("arbitrary",),
                                             vmem_limit_bytes=100 * 1024 * 1024,
                                             disable_bounds_checks=True,
                                             disable_semaphore_checks=True),
    )(A_x.reshape(S, D), A_wqkv, A_wo, B_w_gate, B_w_up, B_w_down)
    return out.reshape(1, S, D)
```
